```python
import jax
import jax.numpy as jnp

def _softmax(x, axis=-1):
    return jax.nn.softmax(x, axis=axis)

def _gelu(x):
    return jax.nn.gelu(x, approximate=True)

def _silu(x):
    return jax.nn.silu(x)

def _sigmoid(x):
    return jax.nn.sigmoid(x)

def _layernorm(x, axis=-1, eps=1e-05):
    m = jnp.mean(x, axis=axis, keepdims=True)
    v = jnp.var(x, axis=axis, keepdims=True)
    return (x - m) / jnp.sqrt(v + eps)

def _scatter_add(tgt, idx, src, axis=0):
    return tgt.at[idx].add(src)

def _segment_sum(src, seg, n):
    return jax.ops.segment_sum(src, seg, n)

class _Rng:

    def __init__(self, key):
        self._k = key

    def _next(self):
        self._k, sub = jax.random.split(self._k)
        return sub

    def normal(self, shape):
        return jax.random.normal(self._next(), shape, dtype=jnp.bfloat16)

    def randint(self, lo, hi, shape):
        return jax.random.randint(self._next(), shape, lo, hi, dtype=jnp.int32)

    def uniform(self, shape, lo=0.0, hi=1.0):
        return jax.random.uniform(self._next(), shape, jnp.bfloat16, lo, hi)

    def permutation(self, n):
        return jax.random.permutation(self._next(), n)
kernel_name = 'sequential_preLN__memory_aug_recurrent_mem_tr__moe_arch_mod__prompt'

def setup_inputs():
    _rng = _Rng(jax.random.key(int.from_bytes(__import__("os").urandom(4), "little")))
    _w = lambda a: (lambda t: t.astype(jnp.bfloat16) if jnp.issubdtype(t.dtype, jnp.floating) else t)(jnp.asarray(a))

    def _A_setup():
        B, S, Dm = (1, 2048, 512)
        H, Dh = (32, 128)
        M, seg = (8, 32)
        seg = min(seg, S)
        S = S // seg * seg
        return {'x': _w((lambda *s: _rng.normal(s) * 0.05)(B, S, Dm)), 'mem0': _w((lambda *s: _rng.normal(s) * 0.05)(B, M, Dm)), 'Wq': _w((lambda *s: _rng.normal(s) * 0.05)(Dm, H, Dh) * Dm ** (-0.5)), 'Wk': _w((lambda *s: _rng.normal(s) * 0.05)(Dm, H, Dh) * Dm ** (-0.5)), 'Wv': _w((lambda *s: _rng.normal(s) * 0.05)(Dm, H, Dh) * Dm ** (-0.5)), 'Wo': _w((lambda *s: _rng.normal(s) * 0.05)(H, Dh, Dm) * (H * Dh) ** (-0.5)), 'seg_len': seg}
    _A_in = _A_setup()

    def _B_setup():
        B, S, D, F, C = (1, 2048, 512, 1792, 2)
        return {'x': _w((lambda *s: _rng.normal(s) * 0.05)(B, S, D)), 'w_r': _w((lambda *s: _rng.normal(s) * 0.05)(D)), 'w_gate': _w((lambda *s: _rng.normal(s) * 0.05)(D, F)), 'w_up': _w((lambda *s: _rng.normal(s) * 0.05)(D, F)), 'w_down': _w((lambda *s: _rng.normal(s) * 0.05)(F, D))}
    _B_in = _B_setup()
    return {'A_x': _A_in['x'], 'A_mem0': _A_in['mem0'], 'A_Wq': _A_in['Wq'], 'A_Wk': _A_in['Wk'], 'A_Wv': _A_in['Wv'], 'A_Wo': _A_in['Wo'], 'A_seg_len': _A_in['seg_len'], 'B_x': _B_in['x'], 'B_w_r': _B_in['w_r'], 'B_w_gate': _B_in['w_gate'], 'B_w_up': _B_in['w_up'], 'B_w_down': _B_in['w_down']}

def reference(A_x, A_mem0, A_Wq, A_Wk, A_Wv, A_Wo, A_seg_len, B_x, B_w_r, B_w_gate, B_w_up, B_w_down):

    def _A_ref(x, mem0, Wq, Wk, Wv, Wo, seg_len):
        B, S, Dm = x.shape
        H, Dh = (Wq.shape[1], Wq.shape[2])
        M = mem0.shape[1]
        scale = Dh ** (-0.5)
        n_seg = S // seg_len
        L = M + seg_len
        idx = jnp.arange(L)
        mask = (idx[:, None] < M) | (idx[:, None] >= idx[None, :])
        mem = mem0
        outs = []
        for s in range(n_seg):
            xs = x[:, s * seg_len:(s + 1) * seg_len, :].copy()
            h = jnp.concatenate([mem, xs], axis=1)
            q = jnp.einsum('btd,dhe->bhte', h, Wq)
            k = jnp.einsum('btd,dhe->bhte', h, Wk)
            v = jnp.einsum('btd,dhe->bhte', h, Wv)
            scores = jnp.einsum('bhqe,bhke->bhqk', q, k) * scale
            scores = jnp.where(mask[None, None], scores, -1000000000.0)
            p = _softmax(scores, axis=-1)
            o = jnp.einsum('bhqk,bhke->bhqe', p, v)
            o = jnp.einsum('bhte,hed->btd', o, Wo)
            mem = o[:, :M, :].copy()
            outs.append(o[:, M:, :])
        return jnp.concatenate(outs, axis=1)

    def _B_ref(x, w_r, w_gate, w_up, w_down):
        B, S, D = x.shape
        C = 2
        r = x @ w_r
        idx = jnp.argsort(-r, axis=-1)[:, :C]
        idx_e = jnp.repeat(idx.reshape(B, C, 1), D, axis=2)
        x_sel = jnp.take_along_axis(x, idx_e, axis=1)
        g = _silu(x_sel @ w_gate)
        u = x_sel @ w_up
        y = g * u @ w_down
        r_sel = _sigmoid(jnp.take_along_axis(r, idx, axis=1))
        y = y * r_sel.reshape(B, C, 1)
        b_off = (jnp.arange(B) * S).reshape(B, 1)
        flat_idx = (idx + b_off).reshape(B * C)
        zero = (x * 0.0).reshape(B * S, D)
        upd = _scatter_add(zero, flat_idx, y.reshape(B * C, D), axis=0)
        return x + upd.reshape(B, S, D)
    x = A_x
    h = x + _A_ref(_layernorm(x, axis=-1), A_mem0, A_Wq, A_Wk, A_Wv, A_Wo, A_seg_len)
    h2 = h + _B_ref(_layernorm(h, axis=-1), B_w_r, B_w_gate, B_w_up, B_w_down)
    return h2
```

```python
import functools
import math

import jax
import jax.numpy as jnp
import numpy as np
from jax import lax
import jax.experimental.pallas as pl
import jax.experimental.pallas.tpu as pltpu

F32 = jnp.float32
BF16 = jnp.bfloat16
LANES = 128


def _rb(v):
    return v.astype(BF16).astype(F32)


def _layernorm(v):
    n = v.shape[-1]
    mean = jnp.sum(v, axis=-1, keepdims=True) * (1.0 / n)
    c = v - mean
    var = jnp.sum(c * c, axis=-1, keepdims=True) * (1.0 / n)
    eps = float(np.asarray(1e-5, dtype=BF16))
    den = _rb(jnp.sqrt(_rb(_rb(var) + eps)))
    return _rb(_rb(v - _rb(mean)) / den)


def _kernel(x_hbm, mem0_ref, wq_hbm, wk_hbm, wv_hbm, wo_hbm, wr_ref, wg_hbm, wu_hbm, wd_hbm,
            out_hbm,
            x_v, raw_q, raw_k, raw_v, w_v, wo_v, wg_v, wu_v, wd_v, xn_v, h_v, o_v, att_v, r_v, cap_v,
            out_v, sems, *, S, D, H, Dh, M, SEG, F, cfg):
    L = M + SEG
    NSEG = S // SEG
    G = cfg.get("G", 3)
    scale = Dh ** -0.5
    NCH = 4
    rows_c = D * H // NCH

    si = [0]

    def new_copy(src, dst):
        c = pltpu.make_async_copy(src, dst, sems.at[si[0]])
        si[0] += 1
        return c

    cp_x = new_copy(x_hbm, x_v)
    cp_w = [[new_copy(w.at[pl.ds(c * rows_c, rows_c), :], r.at[pl.ds(c * rows_c, rows_c), :])
             for c in range(NCH)] for w, r in ((wq_hbm, raw_q), (wk_hbm, raw_k), (wv_hbm, raw_v))]
    cp_o = [new_copy(wo_hbm.at[:, pl.ds(n * LANES, LANES)], wo_v.at[n]) for n in range(D // LANES)]
    cp_f = [new_copy(wg_hbm, wg_v), new_copy(wu_hbm, wu_v), new_copy(wd_hbm, wd_v)]
    queue = [cp_x] + [c for cs in cp_w for c in cs] + cp_o + cp_f
    AHEAD = 3
    for c in queue[:AHEAD]:
        c.start()
    qi = [0]

    def wait_next():
        queue[qi[0]].wait()
        if qi[0] + AHEAD < len(queue):
            queue[qi[0] + AHEAD].start()
        qi[0] += 1

    ri = lax.broadcasted_iota(jnp.int32, (L, LANES), 0)
    ci = lax.broadcasted_iota(jnp.int32, (L, LANES), 1)
    for g in range(G):
        cj = ci - g * L
        own = (cj >= 0) & (cj < L)
        keep = own & ((ri < M) | (ri >= cj))
        cap_v[pl.ds(g * L, L), :] = jnp.where(keep, 1.0, jnp.where(own, -1e9 / scale, -jnp.inf)).astype(F32)
    r_v[...] = jnp.full(r_v.shape, -jnp.inf, F32)
    att_v[...] = jnp.zeros(att_v.shape, F32)

    wait_next()

    def ln_body(i, c):
        r0 = pl.multiple_of(i * 64, 64)
        xn_v[pl.ds(r0, 64), :] = _layernorm(x_v[pl.ds(r0, 64), :].astype(F32))
        return c

    lax.fori_loop(0, S // 64, ln_body, 0)

    HP = H // 2
    DC = 32
    for m, raw in enumerate((raw_q, raw_k, raw_v)):
        ru = raw.bitcast(jnp.uint32)
        for c in range(NCH):
            wait_next()

            def rl_body(i, carry, ru=ru, m=m):
                v = ru.at[pl.ds(pl.multiple_of(i * DC * HP, DC * HP), DC * HP), :]
                d0 = pl.multiple_of(i * DC, DC)
                for j in range(HP):
                    w = v[pl.ds(j, DC, stride=HP), :]
                    lo = pltpu.bitcast(w << 16, F32).astype(BF16)
                    hi = pltpu.bitcast(w & jnp.uint32(0xFFFF0000), F32).astype(BF16)
                    w_v[(2 * j) * 3 + m, pl.ds(d0, DC), :] = lo
                    w_v[(2 * j + 1) * 3 + m, pl.ds(d0, DC), :] = hi
                return carry

            n_it = D // DC // NCH
            lax.fori_loop(c * n_it, (c + 1) * n_it, rl_body, 0)
    for _ in cp_o:
        wait_next()

    wr = wr_ref[...].astype(F32)
    lane_id = lax.broadcasted_iota(jnp.int32, (SEG, LANES), 1)

    def post(s):
        r0 = pl.multiple_of(s * SEG, SEG)
        h = _rb(x_v[pl.ds(r0, SEG), :].astype(F32) + _rb(att_v[...]))
        hn = _layernorm(h)
        h_v[pl.ds(r0, SEG), :] = h
        out_v[pl.ds(r0, SEG), :] = (h + hn).astype(BF16)
        r = _rb(jnp.sum(hn * wr, axis=-1, keepdims=True))
        r_v[...] = jnp.where(lane_id == s, r, r_v[...])

    groups = [list(range(a, min(a + G, H))) for a in range(0, H, G)]
    c_exp = scale * math.log2(math.e)

    def step(s, mem):
        post(jnp.maximum(s - 1, 0))
        r0 = pl.multiple_of(s * SEG, SEG)
        hh = jnp.concatenate([mem, xn_v[pl.ds(r0, SEG), :]], axis=0)

        def proj(g):
            out = []
            for m in range(3):
                out.append([jnp.dot(hh, w_v[hd * 3 + m], preferred_element_type=F32) for hd in g])
            return out

        def scores(g, qkv):
            qs, ks, vs = qkv
            n = len(g)
            pad = [jnp.zeros((LANES - n * L, Dh), F32)]
            q = jnp.concatenate(qs, axis=0)
            k = jnp.concatenate(ks + pad, axis=0).astype(BF16)
            v = jnp.concatenate(vs + pad, axis=0).astype(BF16)
            sc = lax.dot_general(q, k, (((1,), (1,)), ((), ())), preferred_element_type=F32)
            cap = cap_v[pl.ds(0, n * L), :]
            sc = jnp.where(cap > 0.0, sc, cap)
            e = jnp.exp2((sc - jnp.max(sc, axis=-1, keepdims=True)) * c_exp)
            return e, v

        def pv(g, ev):
            e, v = ev
            o = jnp.dot(e, v, preferred_element_type=F32) * (1.0 / jnp.sum(e, axis=-1, keepdims=True))
            for i, hd in enumerate(g):
                o_v[:, pl.ds(hd * Dh, Dh)] = o[i * L:(i + 1) * L]

        ng = len(groups)
        lag1, lag2 = cfg.get("lag1", 1), cfg.get("lag2", 2)
        st1, st2 = {}, {}
        for t in range(ng + lag2):
            if t < ng:
                st1[t] = proj(groups[t])
            if 0 <= t - lag1 < ng:
                st2[t - lag1] = scores(groups[t - lag1], st1.pop(t - lag1))
            if 0 <= t - lag2 < ng:
                pv(groups[t - lag2], st2.pop(t - lag2))
        KS = cfg.get("KS", 8)
        kc = H * Dh // KS
        acc = [None] * (D // LANES)
        for kk in range(KS):
            oo = o_v[:, pl.ds(kk * kc, kc)]
            for n in range(D // LANES):
                d = jnp.dot(oo, wo_v[n, pl.ds(kk * kc, kc), :], preferred_element_type=F32)
                acc[n] = d if acc[n] is None else acc[n] + d
        y = jnp.concatenate(acc, axis=1)
        att_v[...] = y[M:]
        return y[:M]

    lax.fori_loop(0, NSEG, step, mem0_ref[...].astype(F32))
    post(NSEG - 1)

    r = r_v[...]
    tok = lane_id * SEG + lax.broadcasted_iota(jnp.int32, (SEG, LANES), 0)
    big = jnp.int32(2 ** 30)
    valid = lane_id < NSEG
    m1 = jnp.max(r)
    i1 = jnp.min(jnp.where(valid & (r == m1), tok, big))
    valid2 = valid & (tok != i1)
    r2 = jnp.where(valid2, r, -jnp.inf)
    m2 = jnp.max(r2)
    i2 = jnp.min(jnp.where(valid2 & (r2 == m2), tok, big))
    i1 = jnp.clip(i1, 0, S - 1)
    i2 = jnp.clip(i2, 0, S - 1)
    row8 = lax.broadcasted_iota(jnp.int32, (8, D), 0)
    hs = jnp.where(row8 == 0, h_v[pl.ds(i1, 1), :], h_v[pl.ds(i2, 1), :])
    xs = _layernorm(hs)
    for c in cp_f:
        c.wait()
    gg = _rb(jnp.dot(xs, wg_v[...], preferred_element_type=F32))
    uu = _rb(jnp.dot(xs, wu_v[...], preferred_element_type=F32))
    act = _rb(_rb(gg * jax.nn.sigmoid(gg)) * uu)
    y = _rb(jnp.dot(act, wd_v[...], preferred_element_type=F32))
    rs = jnp.where(row8 == 0, m1, m2)
    y = _rb(y * _rb(jax.nn.sigmoid(rs)))
    fin = hs + _rb(xs + y)
    row16 = lax.broadcasted_iota(jnp.int32, (16, D), 0)
    for j, idx in enumerate((i1, i2)):
        b0 = pl.multiple_of((idx // 16) * 16, 16)
        cur = out_v[pl.ds(b0, 16), :].astype(F32)
        out_v[pl.ds(b0, 16), :] = jnp.where(row16 == idx - b0, fin[j:j + 1], cur).astype(BF16)
    cp = new_copy(out_v, out_hbm)
    cp.start()
    cp.wait()


def build(cfg):
    def fn(A_x, A_mem0, A_Wq, A_Wk, A_Wv, A_Wo, A_seg_len, B_x, B_w_r, B_w_gate, B_w_up, B_w_down):
        B, S, D = A_x.shape
        _, H, Dh = A_Wq.shape
        M = A_mem0.shape[1]
        F = B_w_gate.shape[1]
        SEG = int(A_seg_len)
        L = M + SEG
        anyspec = pl.BlockSpec(memory_space=pl.ANY)
        vspec = pl.BlockSpec(memory_space=pltpu.VMEM)
        out = pl.pallas_call(
            functools.partial(_kernel, S=S, D=D, H=H, Dh=Dh, M=M, SEG=SEG, F=F, cfg=cfg),
            out_shape=jax.ShapeDtypeStruct((S, D), BF16),
            in_specs=[anyspec, vspec, anyspec, anyspec, anyspec, anyspec, vspec, anyspec, anyspec, anyspec],
            out_specs=anyspec,
            scratch_shapes=[
                pltpu.VMEM((S, D), BF16),
                pltpu.VMEM((D * H, Dh), BF16), pltpu.VMEM((D * H, Dh), BF16), pltpu.VMEM((D * H, Dh), BF16),
                pltpu.VMEM((3 * H, D, Dh), BF16),
                pltpu.VMEM((D // LANES, H * Dh, LANES), BF16),
                pltpu.VMEM((D, F), BF16), pltpu.VMEM((D, F), BF16), pltpu.VMEM((F, D), BF16),
                pltpu.VMEM((S, D), F32), pltpu.VMEM((S, D), F32),
                pltpu.VMEM((L, H * Dh), F32), pltpu.VMEM((SEG, D), F32), pltpu.VMEM((SEG, LANES), F32),
                pltpu.VMEM((3 * L, LANES), F32),
                pltpu.VMEM((S, D), BF16),
                pltpu.SemaphoreType.DMA((32,)),
            ],
            compiler_params=pltpu.CompilerParams(vmem_limit_bytes=100 * 1024 * 1024, flags=cfg.get("flags")),
            name="rmt",
        )(A_x.reshape(S, D), A_mem0.reshape(M, D), A_Wq.reshape(D * H, Dh), A_Wk.reshape(D * H, Dh),
          A_Wv.reshape(D * H, Dh), A_Wo.reshape(H * Dh, D), B_w_r.reshape(1, D), B_w_gate, B_w_up, B_w_down)
        return out.reshape(B, S, D)
    return fn


@functools.partial(jax.jit, static_argnames=("A_seg_len",))
def pallas_sequential_preLN__memory_aug_recurrent_mem_tr__moe_arch_mod__prompt_kernel(
        A_x, A_mem0, A_Wq, A_Wk, A_Wv, A_Wo, A_seg_len, B_x, B_w_r, B_w_gate, B_w_up, B_w_down):
    return build({})(A_x, A_mem0, A_Wq, A_Wk, A_Wv, A_Wo, A_seg_len, B_x, B_w_r, B_w_gate, B_w_up, B_w_down)
```

```python
import contextlib
import functools
import math

import jax
import jax.numpy as jnp
import numpy as np
from jax import lax
import jax.experimental.pallas as pl
import jax.experimental.pallas.tpu as pltpu

F32 = jnp.float32
BF16 = jnp.bfloat16
U32 = jnp.uint32
LANES = 128


def _rb(v):
    return v.astype(BF16).astype(F32)


def _layernorm(v):
    n = v.shape[-1]
    mean = jnp.sum(v, axis=-1, keepdims=True) * (1.0 / n)
    c = v - mean
    var = jnp.sum(c * c, axis=-1, keepdims=True) * (1.0 / n)
    eps = float(np.asarray(1e-5, dtype=BF16))
    den = _rb(jnp.sqrt(_rb(_rb(var) + eps)))
    return _rb(_rb(v - _rb(mean)) / den)


def _mm(a, b):
    return jnp.dot(a, b, preferred_element_type=F32)


def _kernel(x_hbm, mem0_hbm, wq_hbm, wk_hbm, wv_hbm, wo_hbm, wr_hbm, wg_hbm, wu_hbm, wd_hbm,
            out_hbm,
            mem0_v, wr_v, xa_v, xan_v, x_v, raw_v, w_v, pre_v, wo_v, wg_v, wu_v, wd_v, h_v, att_v, r_v, cap_v,
            out_v, wsem, sems, *, S, D, H, Dh, M, SEG, F, cfg):
    SC = jax.named_scope if cfg.get('scopes') else (lambda n: contextlib.nullcontext())
    L = M + SEG
    NSEG = S // SEG
    G = cfg.get("G", 3)
    P = 8
    NPRE = cfg.get("NPRE", 3)
    HP = H // 2
    XO = 3 * H * P
    scale = Dh ** -0.5

    si = [0]

    def new_copy(src, dst):
        c = pltpu.make_async_copy(src, dst, sems.at[si[0]])
        si[0] += 1
        return c

    cp_xa = new_copy(x_hbm.at[:, pl.ds(0, P), :], xa_v)
    cp_small = [new_copy(mem0_hbm, mem0_v), new_copy(wr_hbm, wr_v)]
    hs_ = NSEG // 2
    cp_x = [new_copy(x_hbm.at[pl.ds(a * hs_, hs_)], x_v.at[pl.ds(a * hs_, hs_)]) for a in range(2)]
    cp_o = [new_copy(wo_hbm.at[:, pl.ds(n * LANES, LANES)], wo_v.bitcast(BF16).at[n]) for n in range(D // LANES)]
    cp_f = [new_copy(wg_hbm, wg_v), new_copy(wu_hbm, wu_v), new_copy(wd_hbm, wd_v)]
    w_hbm = (wq_hbm, wk_hbm, wv_hbm)
    PPI = cfg.get("PPI", 2)
    NIT = HP // PPI
    vfull = cfg.get("vfull", ())

    def ahead(hd, m):
        return m < 2 or (hd % 2) not in vfull

    def start_units(a, b):
        for k in range(a, b):
            j, m = divmod(k, 3)
            pltpu.make_async_copy(w_hbm[m].bitcast(U32).at[:, j, :], raw_v.at[k], wsem.at[k]).start()

    def start_iter(i):
        start_units(i * PPI * 3, (i + 1) * PPI * 3)

    U0, U1 = cfg.get("U0", 0), cfg.get("U1", 3)
    cp_xa.start()
    start_units(0, U0)

    ri = lax.broadcasted_iota(jnp.int32, (L, LANES), 0)
    ci = lax.broadcasted_iota(jnp.int32, (L, LANES), 1)
    for g in range(G):
        cj = ci - g * L
        own = (cj >= 0) & (cj < L)
        keep = own & ((ri < M) | (ri >= cj))
        cap_v[pl.ds(g * L, L), :] = jnp.where(keep, 1.0, jnp.where(own, -1e9 / scale, -jnp.inf)).astype(F32)
    r_v[...] = jnp.full(r_v.shape, -jnp.inf, F32)
    att_v[...] = jnp.zeros(att_v.shape, F32)

    with SC('w_xa'):
        cp_xa.wait()
    start_units(U0, U1)
    LB = cfg.get("LB", 16)

    def ln_body(i, c):
        s0 = pl.multiple_of(i * LB, LB)
        v = xa_v[pl.ds(s0, LB)].astype(F32).reshape(LB * P, D)
        r0 = pl.multiple_of(i * (LB * P // 2), LB * P // 2)
        xan_v[pl.ds(r0, LB * P // 2), :] = pltpu.bitcast(_layernorm(v).astype(BF16), U32)
        return c

    with SC('ln_a'):
        lax.fori_loop(0, NSEG // LB, ln_body, 0)

    extra = cp_small + cp_x + cp_o
    phases = cfg.get("phases", ((1, 2), (2, 7)))
    bounds = [0]
    for ppi, nit in phases:
        bounds += [bounds[-1] + ppi * (c + 1) for c in range(nit)]
    assert bounds[-1] == HP
    n_all = len(bounds) - 1
    started = [U1]
    XS = cfg.get("XS", 3)

    def start_more(g):
        upto = 3 * bounds[min(g + (2 if g < cfg.get("G2", 2) else 3), n_all)]
        start_units(started[0], upto)
        started[0] = max(started[0], upto)
        for n, e in enumerate(extra):
            if XS + n * (n_all - 1 - XS) // len(extra) == g:
                e.start()

    g0 = 0
    for ppi, nit in phases:
        p0 = bounds[g0]

        def pre_body(i, carry, ppi=ppi, nit=nit, p0=p0, g0=g0):
            with SC('w_w'):
                for u in range(ppi * 3):
                    k = (p0 + i * ppi) * 3 + u
                    pltpu.make_async_copy(raw_v.at[k], raw_v.at[k], wsem.at[k]).wait()
            for c in range(nit):
                pl.when(i == c)(functools.partial(start_more, g0 + c))
            for u in range(ppi):
                for m in range(3):
                    j = p0 + i * ppi + u
                    w = raw_v[j * 3 + m]
                    lo = pltpu.bitcast(w << 16, F32).astype(BF16)
                    hi = pltpu.bitcast(w & U32(0xFFFF0000), F32).astype(BF16)
                    for t, wt in enumerate((lo, hi)):
                        hm = (2 * j + t) * 3 + m
                        w_v[hm] = pltpu.bitcast(wt, U32)
                        if ahead(t, m):
                            d = _mm(pltpu.bitcast(xan_v[...], BF16), wt)
                            pre_v[:, pl.ds(pl.multiple_of(hm * P, P), P), :] = d.reshape(NSEG, P, Dh)
            return carry

        with SC('pre'):
            lax.fori_loop(0, nit, pre_body, 0)
        g0 += nit
    with SC('w_o'):
        for c in cp_small + cp_x + cp_o:
            c.wait()
    for c in cp_f:
        c.start()

    def pre_ln(s):
        v = _layernorm(x_v[s].astype(F32))
        for n in range(D // LANES):
            pre_v[s, pl.ds(XO + n * SEG, SEG), :] = v[:, n * LANES:(n + 1) * LANES]

    pre_ln(0)
    wr = wr_v[...].astype(F32).reshape(1, D)
    lane_id = lax.broadcasted_iota(jnp.int32, (SEG, LANES), 1)

    def post(s):
        r0 = pl.multiple_of(s * SEG, SEG)
        h = _rb(x_v[s].astype(F32) + _rb(att_v[...]))
        hn = _layernorm(h)
        h_v[pl.ds(r0, SEG), :] = h
        out_v[pl.ds(r0, SEG), :] = (h + hn).astype(BF16)
        r = _rb(jnp.sum(hn * wr, axis=-1, keepdims=True))
        r_v[...] = jnp.where(lane_id == s, r, r_v[...])

    gsz = cfg.get("gsz", [3] * 10 + [2])
    groups, a = [], 0
    for n in gsz:
        groups.append(list(range(a, a + n)))
        a += n
    assert a == H
    c_exp = scale * math.log2(math.e)
    UN = cfg.get('UN', 1)
    EARLY = NSEG - max(UN, 2)
    cp_out0 = new_copy(out_v.at[pl.ds(0, (EARLY - 1) * SEG)], out_hbm.at[pl.ds(0, (EARLY - 1) * SEG)])
    cp_out1 = new_copy(out_v.at[pl.ds((EARLY - 1) * SEG, S - (EARLY - 1) * SEG)],
                       out_hbm.at[pl.ds((EARLY - 1) * SEG, S - (EARLY - 1) * SEG)])

    def step(s, mem):
        xs_ = jnp.concatenate([pre_v[s, pl.ds(XO + n * SEG, SEG), :] for n in range(D // LANES)], axis=1)
        h_full = jnp.concatenate([xs_, mem], axis=0)
        h_part = jnp.concatenate([xs_[P:], mem], axis=0)
        if cfg.get("lhs16", True):
            h_part = h_part.astype(BF16)
        pr, ev, oh = {}, {}, {}
        acc = [None] * (D // LANES)

        def proj(hd, m):
            w = pltpu.bitcast(w_v[hd * 3 + m], BF16)
            if ahead(hd, m):
                d = _mm(h_part, w)
                pr[hd, m] = jnp.concatenate(
                    [d[SEG - P:], pre_v[s, pl.ds((hd * 3 + m) * P, P), :], d[:SEG - P]], axis=0)
            else:
                d = _mm(h_full, w)
                pr[hd, m] = jnp.concatenate([d[SEG:], d[:SEG]], axis=0)

        def scores(t):
            g = groups[t]
            n = len(g)
            pad = [jnp.zeros((LANES - n * L, Dh), F32)]
            q = jnp.concatenate([pr.pop((hd, 0)) for hd in g], axis=0)
            k = jnp.concatenate([pr.pop((hd, 1)) for hd in g] + pad, axis=0).astype(BF16)
            sc = lax.dot_general(q, k, (((1,), (1,)), ((), ())), preferred_element_type=F32)
            cap = cap_v[pl.ds(0, n * L), :]
            sc = jnp.where(cap > 0.0, sc, cap)
            ev[t] = jnp.exp2((sc - jnp.max(sc, axis=-1, keepdims=True)) * c_exp)

        def pv(t):
            g = groups[t]
            pad = [jnp.zeros((LANES - len(g) * L, Dh), F32)]
            v = jnp.concatenate([pr.pop((hd, 2)) for hd in g] + pad, axis=0).astype(BF16)
            e = ev.pop(t)
            o = _mm(e, v) * (1.0 / jnp.sum(e, axis=-1, keepdims=True))
            for i, hd in enumerate(g):
                oh[hd] = o[i * L:(i + 1) * L]

        wo_done = [0]

        def wo(nh):
            h0 = wo_done[0]
            oo = jnp.concatenate([oh.pop(hd) for hd in range(h0, h0 + nh)], axis=1)
            for n in range(D // LANES):
                d = _mm(oo, pltpu.bitcast(wo_v[n, pl.ds(h0 * Dh // 2, nh * Dh // 2), :], BF16))
                acc[n] = d if acc[n] is None else acc[n] + d
            wo_done[0] = h0 + nh

        for op in cfg["prog"](groups):
            if op[0] == "P":
                proj(op[1], op[2])
            elif op[0] == "S":
                scores(op[1])
            elif op[0] == "V":
                pv(op[1])
            elif op[0] == "O":
                wo(op[1])
            elif op[0] == "ln":
                pre_ln(jnp.minimum(s + 1, NSEG - 1))
            elif op[0] == "post":
                post(jnp.maximum(s - 1, 0))
        assert wo_done[0] == H
        y = jnp.concatenate(acc, axis=1)
        att_v[...] = y[M:]
        return y[:M]

    def steps(i, mem):
        @pl.when(i == EARLY // UN)
        def _():
            cp_out0.start()

        for u in range(UN):
            mem = step(i * UN + u, mem)
        return mem

    with SC('main'):
        lax.fori_loop(0, NSEG // UN, steps, mem0_v[...].astype(F32))
    post(NSEG - 1)
    cp_out1.start()

    r = r_v[...]
    tok = lane_id * SEG + lax.broadcasted_iota(jnp.int32, (SEG, LANES), 0)
    big = jnp.int32(2 ** 30)
    valid = lane_id < NSEG
    m1 = jnp.max(r)
    i1 = jnp.min(jnp.where(valid & (r == m1), tok, big))
    valid2 = valid & (tok != i1)
    r2 = jnp.where(valid2, r, -jnp.inf)
    m2 = jnp.max(r2)
    i2 = jnp.min(jnp.where(valid2 & (r2 == m2), tok, big))
    i1 = jnp.clip(i1, 0, S - 1)
    i2 = jnp.clip(i2, 0, S - 1)
    row8 = lax.broadcasted_iota(jnp.int32, (8, D), 0)
    hs = jnp.where(row8 == 0, h_v[pl.ds(i1, 1), :], h_v[pl.ds(i2, 1), :])
    xs = _layernorm(hs)
    for c in cp_f:
        c.wait()
    gg = _rb(_mm(xs, wg_v[...]))
    uu = _rb(_mm(xs, wu_v[...]))
    act = _rb(_rb(gg * jax.nn.sigmoid(gg)) * uu)
    y = _rb(_mm(act, wd_v[...]))
    rs = jnp.where(row8 == 0, m1, m2)
    y = _rb(y * _rb(jax.nn.sigmoid(rs)))
    fin = hs + _rb(xs + y)
    with SC('w_out'):
        cp_out0.wait()
        cp_out1.wait()
    row16 = lax.broadcasted_iota(jnp.int32, (16, D), 0)
    bs = []
    for j, idx in enumerate((i1, i2)):
        b0 = pl.multiple_of((idx // 16) * 16, 16)
        cur = out_v[pl.ds(b0, 16), :].astype(F32)
        out_v[pl.ds(b0, 16), :] = jnp.where(row16 == idx - b0, fin[j:j + 1], cur).astype(BF16)
        bs.append(b0)
    fix = [new_copy(out_v.at[pl.ds(b0, 16)], out_hbm.at[pl.ds(b0, 16)]) for b0 in bs]
    fix[0].start()

    @pl.when(bs[0] != bs[1])
    def _():
        fix[1].start()
        fix[1].wait()

    with SC('w_fix'):
        fix[0].wait()


def prog(vlag=1, wo=None, postat=0, lnat=3, wc=2, korder=(1, 0)):
    wo = wo or {}

    def f(groups):
        ng = len(groups)
        out = []
        done = [0]

        def O(upto):
            while done[0] < upto:
                n = min(wc, upto - done[0])
                out.append(("O", n))
                done[0] += n

        for t in range(ng + 2):
            if t == postat:
                out.append(("post",))
            if t == lnat:
                out.append(("ln",))
            if t < ng:
                for m in korder:
                    out.extend(("P", hd, m) for hd in groups[t])
            if vlag == 0 and t < ng:
                out.extend(("P", hd, 2) for hd in groups[t])
            if t in wo:
                O(wo[t][0])
            if vlag == 1.5 and 0 <= t - 1 < ng:
                out.extend(("P", hd, 2) for hd in groups[t - 1])
            if 0 <= t - 1 < ng:
                out.append(("S", t - 1))
            if vlag == 1 and 0 <= t - 1 < ng:
                out.extend(("P", hd, 2) for hd in groups[t - 1])
            if t in wo:
                O(wo[t][1])
            if 0 <= t - 2 < ng:
                out.append(("V", t - 2))
        O(sum(len(g) for g in groups))
        return out
    return f


def build(cfg):
    cfg = dict(cfg)
    cfg["prog"] = prog(**cfg.get("p", dict(wo={11: (4, 8), 12: (16, 16)})))

    def fn(A_x, A_mem0, A_Wq, A_Wk, A_Wv, A_Wo, A_seg_len, B_x, B_w_r, B_w_gate, B_w_up, B_w_down):
        B, S, D = A_x.shape
        _, H, Dh = A_Wq.shape
        M = A_mem0.shape[1]
        F = B_w_gate.shape[1]
        SEG = int(A_seg_len)
        NSEG = S // SEG
        L = M + SEG
        anyspec = pl.BlockSpec(memory_space=pl.ANY)
        vspec = pl.BlockSpec(memory_space=pltpu.VMEM)
        out = pl.pallas_call(
            functools.partial(_kernel, S=S, D=D, H=H, Dh=Dh, M=M, SEG=SEG, F=F, cfg=cfg),
            out_shape=jax.ShapeDtypeStruct((S, D), BF16),
            in_specs=[anyspec] * 10,
            out_specs=anyspec,
            scratch_shapes=[
                pltpu.VMEM((M, D), BF16), pltpu.VMEM((D,), BF16),
                pltpu.VMEM((NSEG, 8, D), BF16),
                pltpu.VMEM((NSEG * 8 // 2, D), U32),
                pltpu.VMEM((NSEG, SEG, D), BF16),
                pltpu.VMEM((3 * H // 2, D, Dh), U32),
                pltpu.VMEM((3 * H, D // 2, Dh), U32),
                pltpu.VMEM((NSEG, 3 * H * 8 + SEG * D // LANES, Dh), F32),
                pltpu.VMEM((D // LANES, H * Dh // 2, LANES), U32),
                pltpu.VMEM((D, F), BF16), pltpu.VMEM((D, F), BF16), pltpu.VMEM((F, D), BF16),
                pltpu.VMEM((S, D), F32),
                pltpu.VMEM((SEG, D), F32), pltpu.VMEM((SEG, LANES), F32),
                pltpu.VMEM((3 * L, LANES), F32),
                pltpu.VMEM((S, D), BF16),
                pltpu.SemaphoreType.DMA((3 * H // 2,)),
                pltpu.SemaphoreType.DMA((20,)),
            ],
            compiler_params=pltpu.CompilerParams(vmem_limit_bytes=100 * 1024 * 1024, flags=cfg.get("flags")),
            name="rmt",
        )(A_x.reshape(NSEG, SEG, D), A_mem0.reshape(M, D), A_Wq, A_Wk, A_Wv, A_Wo.reshape(H * Dh, D),
          B_w_r, B_w_gate, B_w_up, B_w_down)
        return out.reshape(B, S, D)
    return fn


@functools.partial(jax.jit, static_argnames=("A_seg_len",))
def pallas_sequential_preLN__memory_aug_recurrent_mem_tr__moe_arch_mod__prompt_kernel(
        A_x, A_mem0, A_Wq, A_Wk, A_Wv, A_Wo, A_seg_len, B_x, B_w_r, B_w_gate, B_w_up, B_w_down):
    return build({'U0':1})(A_x, A_mem0, A_Wq, A_Wk, A_Wv, A_Wo, A_seg_len, B_x, B_w_r, B_w_gate, B_w_up, B_w_down)
```

```python
import contextlib
import functools
import math

import jax
import jax.numpy as jnp
import numpy as np
from jax import lax
import jax.experimental.pallas as pl
import jax.experimental.pallas.tpu as pltpu

F32 = jnp.float32
BF16 = jnp.bfloat16
U32 = jnp.uint32
LANES = 128


def _rb(v):
    return v.astype(BF16).astype(F32)


def _layernorm_stages(v, rounded=True):
    n = v.shape[-1]
    mean = jnp.sum(v, axis=-1, keepdims=True) * (1.0 / n)
    yield
    c = v - mean
    var = jnp.sum(c * c, axis=-1, keepdims=True) * (1.0 / n)
    yield
    if not rounded:
        return c * lax.rsqrt(var + 1e-5)
    eps = float(np.asarray(1e-5, dtype=BF16))
    den = _rb(jnp.sqrt(_rb(_rb(var) + eps)))
    return _rb(_rb(v - _rb(mean)) / den)


def _run(gen):
    while True:
        try:
            next(gen)
        except StopIteration as stop:
            return stop.value


def _layernorm(v):
    return _run(_layernorm_stages(v))


def _mm(a, b):
    return jnp.dot(a, b, preferred_element_type=F32)


def _kernel(x_hbm, mem0_hbm, wq_hbm, wk_hbm, wv_hbm, wo_hbm, wr_hbm, wg_hbm, wu_hbm, wd_hbm,
            out_hbm,
            mem0_v, wr_v, xa_v, xan_v, x_v, raw_v, w_v, pre_v, wo_v, wg_v, wu_v, wd_v, h_v, hn_v, att_v, r_v, cap_v,
            out_v, wsem, sems, *, S, D, H, Dh, M, SEG, F, cfg):
    SC = jax.named_scope if cfg.get('scopes') else (lambda n: contextlib.nullcontext())
    L = M + SEG
    NSEG = S // SEG
    G = cfg.get("G", 3)
    P = 8
    NPRE = cfg.get("NPRE", 3)
    HP = H // 2
    XO = 3 * H * P
    scale = Dh ** -0.5

    si = [0]

    def new_copy(src, dst):
        c = pltpu.make_async_copy(src, dst, sems.at[si[0]])
        si[0] += 1
        return c

    cp_xa = new_copy(x_hbm.at[:, pl.ds(0, P), :], xa_v)
    cp_small = [new_copy(mem0_hbm, mem0_v), new_copy(wr_hbm, wr_v)]
    hs_ = NSEG // 2
    cp_x = [new_copy(x_hbm.at[pl.ds(a * hs_, hs_)], x_v.at[pl.ds(a * hs_, hs_)]) for a in range(2)]
    cp_o = [new_copy(wo_hbm.at[:, pl.ds(n * LANES, LANES)], wo_v.bitcast(BF16).at[n]) for n in range(D // LANES)]
    cp_f = [new_copy(wg_hbm, wg_v), new_copy(wu_hbm, wu_v), new_copy(wd_hbm, wd_v)]
    w_hbm = (wq_hbm, wk_hbm, wv_hbm)
    PPI = cfg.get("PPI", 2)
    NIT = HP // PPI
    vfull = cfg.get("vfull", ())

    def ahead(hd, m):
        return m < 2 or hd >= cfg.get('NV', 0)

    def start_units(a, b):
        for k in range(a, b):
            j, m = divmod(k, 3)
            pltpu.make_async_copy(w_hbm[m].bitcast(U32).at[:, j, :], raw_v.at[k], wsem.at[k]).start()

    def start_iter(i):
        start_units(i * PPI * 3, (i + 1) * PPI * 3)

    U0, U1 = cfg.get("U0", 1), cfg.get("U1", 3)
    cp_xa.start()
    start_units(0, U0)

    ri = lax.broadcasted_iota(jnp.int32, (L, LANES), 0)
    ci = lax.broadcasted_iota(jnp.int32, (L, LANES), 1)
    for g in range(G):
        cj = ci - g * L
        own = (cj >= 0) & (cj < L)
        keep = own & ((ri < M) | (ri >= cj))
        cap_v[pl.ds(g * L, L), :] = jnp.where(keep, 1.0, jnp.where(own, -1e9 / scale, -jnp.inf)).astype(F32)
    r_v[...] = jnp.full(r_v.shape, -1, jnp.int32)
    att_v[...] = jnp.zeros(att_v.shape, F32)

    with SC('w_xa'):
        cp_xa.wait()
    start_units(U0, U1)
    LB = cfg.get("LB", 32)

    def ln_body(i, c):
        s0 = pl.multiple_of(i * LB, LB)
        v = xa_v[pl.ds(s0, LB)].astype(F32).reshape(LB * P, D)
        r0 = pl.multiple_of(i * (LB * P // 2), LB * P // 2)
        xan_v[pl.ds(r0, LB * P // 2), :] = pltpu.bitcast(_run(_layernorm_stages(v, cfg.get('rnd', True))).astype(BF16), U32)
        return c

    with SC('ln_a'):
        lax.fori_loop(0, NSEG // LB, ln_body, 0)

    extra = cp_small + cp_x + cp_o
    phases = cfg.get("phases", ((1, 2), (2, 7)))
    bounds = [0]
    for ppi, nit in phases:
        bounds += [bounds[-1] + ppi * (c + 1) for c in range(nit)]
    assert bounds[-1] == HP
    n_all = len(bounds) - 1
    started = [U1]
    XS = cfg.get("XS", 3)

    def start_more(g):
        upto = 3 * bounds[min(g + (2 if g < cfg.get("G2", 1) else 3), n_all)]
        start_units(started[0], upto)
        started[0] = max(started[0], upto)
        for n, e in enumerate(extra):
            if XS + n * (n_all - 1 - XS) // len(extra) == g:
                e.start()

    g0 = 0
    for ppi, nit in phases:
        p0 = bounds[g0]

        def pre_body(i, carry, ppi=ppi, nit=nit, p0=p0, g0=g0):
            with SC('w_w'):
                for u in range(ppi * 3):
                    k = (p0 + i * ppi) * 3 + u
                    pltpu.make_async_copy(raw_v.at[k], raw_v.at[k], wsem.at[k]).wait()
            for c in range(nit):
                pl.when(i == c)(functools.partial(start_more, g0 + c))
            for u in range(ppi):
                for m in range(3):
                    j = p0 + i * ppi + u
                    w = raw_v[j * 3 + m]
                    lo = pltpu.bitcast(w << 16, F32).astype(BF16)
                    hi = pltpu.bitcast(w & U32(0xFFFF0000), F32).astype(BF16)
                    for t, wt in enumerate((lo, hi)):
                        hm = (2 * j + t) * 3 + m
                        w_v[hm] = pltpu.bitcast(wt, U32)
                        if ahead(2 * p0, m):
                            d = _mm(pltpu.bitcast(xan_v[...], BF16), wt)
                            pre_v[pl.ds(0, NSEG), pl.ds(pl.multiple_of(hm * P, P), P), :] = d.reshape(NSEG, P, Dh)
            return carry

        with SC('pre'):
            lax.fori_loop(0, nit, pre_body, 0)
        g0 += nit
    with SC('w_o'):
        for c in cp_small + cp_x + cp_o:
            c.wait()
    for c in cp_f:
        c.start()

    def pre_ln(s):
        v = yield from _layernorm_stages(x_v[s].astype(F32), cfg.get('rnd', True))
        for n in range(D // LANES):
            pre_v[s, pl.ds(XO + n * SEG, SEG), :] = v[:, n * LANES:(n + 1) * LANES]

    _run(pre_ln(0))
    wr = wr_v[...].astype(F32).reshape(1, D)
    row_id = lax.broadcasted_iota(jnp.int32, (SEG, LANES), 0)

    def post(s, live):
        r0 = pl.multiple_of(s * SEG, SEG)
        h = _rb(x_v[s].astype(F32) + _rb(att_v[...]))
        h_v[pl.ds(r0, SEG), :] = h
        hn = yield from _layernorm_stages(h)
        hn_v[pl.ds(r0, SEG), :] = hn
        out_v[pl.ds(r0, SEG), :] = (h + hn).astype(BF16)
        r = _rb(jnp.sum(hn * wr, axis=-1, keepdims=True))
        r = jnp.broadcast_to(r, (SEG, LANES))
        u = pltpu.bitcast(r, jnp.int32) >> 16
        mono = jnp.where(r == r, (u ^ ((u >> 15) & 0x7FFF)) + 0x8000, 0)
        key = jnp.where(live, mono * S + (S - 1 - r0) - row_id, -1)
        t1 = r_v[0]
        r_v[0] = jnp.maximum(t1, key)
        r_v[1] = jnp.maximum(r_v[1], jnp.minimum(t1, key))

    gsz = cfg.get("gsz", [3] * 10 + [2])
    groups, a = [], 0
    for n in gsz:
        groups.append(list(range(a, a + n)))
        a += n
    assert a == H
    c_exp = scale * math.log2(math.e)
    UN = cfg.get('UN', 1)
    EARLY = NSEG - max(2 * UN, 4)
    cp_out0 = new_copy(out_v.at[pl.ds(0, (EARLY - 1) * SEG)], out_hbm.at[pl.ds(0, (EARLY - 1) * SEG)])
    cp_out1 = new_copy(out_v.at[pl.ds((EARLY - 1) * SEG, S - (EARLY - 1) * SEG)],
                       out_hbm.at[pl.ds((EARLY - 1) * SEG, S - (EARLY - 1) * SEG)])

    def step(s, mem, last):
        xs_ = jnp.concatenate([pre_v[s, pl.ds(XO + n * SEG, SEG), :] for n in range(D // LANES)], axis=1)
        h_full = jnp.concatenate([xs_, mem], axis=0)
        h_part = jnp.concatenate([xs_[P:], mem], axis=0)
        if cfg.get("lhs16", True):
            h_part = h_part.astype(BF16)
        pr, ev, oh = {}, {}, {}
        acc = [None] * (D // LANES)

        def proj(hd, m):
            w = pltpu.bitcast(w_v[hd * 3 + m], BF16)
            if ahead(hd, m):
                d = _mm(h_part, w)
                pr[hd, m] = jnp.concatenate(
                    [d[SEG - P:], pre_v[s, pl.ds((hd * 3 + m) * P, P), :], d[:SEG - P]], axis=0)
            else:
                d = _mm(h_full, w)
                pr[hd, m] = jnp.concatenate([d[SEG:], d[:SEG]], axis=0)

        def scores(t):
            g = groups[t]
            n = len(g)
            pad = [jnp.zeros((LANES - n * L, Dh), F32)]
            q = jnp.concatenate([pr.pop((hd, 0)) for hd in g], axis=0)
            k = jnp.concatenate([pr.pop((hd, 1)) for hd in g] + pad, axis=0).astype(BF16)
            sc = lax.dot_general(q, k, (((1,), (1,)), ((), ())), preferred_element_type=F32)
            cap = cap_v[pl.ds(0, n * L), :]
            sc = jnp.where(cap > 0.0, sc, cap)
            ev[t] = jnp.exp2((sc - jnp.max(sc, axis=-1, keepdims=True)) * c_exp)

        def pv(t):
            g = groups[t]
            pad = [jnp.zeros((LANES - len(g) * L, Dh), F32)]
            v = jnp.concatenate([pr.pop((hd, 2)) for hd in g] + pad, axis=0).astype(BF16)
            e = ev.pop(t)
            den = jnp.sum(e, axis=-1, keepdims=True)
            if cfg.get("rcp", 1):
                inv = pltpu.reciprocal(den, approx=True)
                inv = inv * (2.0 - den * inv)
            else:
                inv = 1.0 / den
            o = _mm(e, v) * inv
            for i, hd in enumerate(g):
                if cfg.get("pin"):
                    pre_v[NSEG + hd // 16, pl.ds((hd % 16) * L, L), :] = o[i * L:(i + 1) * L]
                else:
                    oh[hd] = o[i * L:(i + 1) * L]

        accm = [None] * (D // LANES)
        g_ln = pre_ln(jnp.minimum(s + 1, NSEG - 1))
        g_post = post(jnp.maximum(s - 1, 0), s > 0)

        def add(a, n, d):
            a[n] = d if a[n] is None else a[n] + d

        def wo(h0, nh, part):
            if cfg.get("pin"):
                oo = jnp.concatenate([pre_v[NSEG + hd // 16, pl.ds((hd % 16) * L, L), :]
                                      for hd in range(h0, h0 + nh)], axis=1)
            else:
                oo = jnp.concatenate([oh[hd] for hd in range(h0, h0 + nh)], axis=1)
            oo = {"a": oo, "m": oo[:M], "x": oo[M:]}[part]
            for n in range(D // LANES):
                d = _mm(oo, pltpu.bitcast(wo_v[n, pl.ds(h0 * Dh // 2, nh * Dh // 2), :], BF16))
                if part != "x":
                    add(accm, n, d[:M])
                if part != "m":
                    add(acc, n, d[-SEG:])

        for op in cfg["prog"](groups, last):
            if op[0] == "P":
                proj(op[1], op[2])
            elif op[0] == "S":
                scores(op[1])
            elif op[0] == "V":
                pv(op[1])
            elif op[0] == "O":
                wo(*op[1:])
            elif op[0] == "ln":
                next(g_ln, None)
            elif op[0] == "post":
                next(g_post, None)
        att_v[...] = jnp.concatenate(acc, axis=1)
        return jnp.concatenate(accm, axis=1)

    def steps(i, mem):
        @pl.when(i == EARLY // UN)
        def _():
            cp_out0.start()

        for u in range(UN):
            mem = step(i * UN + u, mem, u == UN - 1)
        return mem

    with SC('main'):
        lax.fori_loop(0, NSEG // UN, steps, mem0_v[...].astype(F32))
    for c in cp_f:
        c.wait()
    _run(post(NSEG - 1, True))
    cp_out1.start()

    t1 = r_v[0]
    k1 = jnp.max(t1, axis=0, keepdims=True)
    k2 = jnp.max(jnp.where(t1 == k1, r_v[1], t1), axis=0, keepdims=True)
    i1 = S - 1 - lax.rem(k1[0, 0], S)
    i2 = S - 1 - lax.rem(k2[0, 0], S)
    row8 = lax.broadcasted_iota(jnp.int32, (8, D), 0)
    hs = jnp.where(row8 == 0, h_v[pl.ds(i1, 1), :], h_v[pl.ds(i2, 1), :])
    xs = jnp.where(row8 == 0, hn_v[pl.ds(i1, 1), :], hn_v[pl.ds(i2, 1), :])
    gg = _rb(_mm(xs, wg_v[...]))
    uu = _rb(_mm(xs, wu_v[...]))
    act = _rb(_rb(gg * jax.nn.sigmoid(gg)) * uu)
    y = _rb(_mm(act, wd_v[...]))
    rs = _rb(jnp.sum(xs * wr, axis=-1, keepdims=True))
    y = _rb(y * _rb(jax.nn.sigmoid(rs)))
    fin = hs + _rb(xs + y)
    with SC('w_out'):
        cp_out0.wait()
        cp_out1.wait()
    row16 = lax.broadcasted_iota(jnp.int32, (16, D), 0)
    bs = []
    for j, idx in enumerate((i1, i2)):
        b0 = pl.multiple_of((idx // 16) * 16, 16)
        cur = out_v[pl.ds(b0, 16), :].astype(F32)
        out_v[pl.ds(b0, 16), :] = jnp.where(row16 == idx - b0, fin[j:j + 1], cur).astype(BF16)
        bs.append(b0)
    fix = [new_copy(out_v.at[pl.ds(b0, 16)], out_hbm.at[pl.ds(b0, 16)]) for b0 in bs]
    fix[0].start()

    @pl.when(bs[0] != bs[1])
    def _():
        fix[1].start()
        fix[1].wait()

    with SC('w_fix'):
        fix[0].wait()


def prog(pat="k0 q0 O S1 v1 O V3", wo={5:(2,2),6:(4,4),7:(6,6),8:(8,8),9:(10,10),10:(12,12),11:(16,16),12:(20,20),13:(24,24)}, postat=(1, 2, 3), lnat=(5, 6, 7), wc=1, split=(22, 26, 30)):
    wo = wo or {}

    def f(groups, last):
        ng = len(groups)
        out = []
        done = [0]
        sp = () if last else split

        def O(upto):
            while done[0] < upto:
                h = done[0]
                if h in sp:
                    out.append(("O", h, 1, "m"))
                    done[0] += 1
                    continue
                n = 1
                while n < wc and h + n < upto and h + n not in sp:
                    n += 1
                out.append(("O", h, n, "a"))
                done[0] += n

        for t in range(ng + 4):
            out.extend(("post",) for a in postat if a == t)
            out.extend(("ln",) for a in lnat if a == t)
            oi = 0
            for tok in pat.split():
                if tok == "O":
                    if t in wo:
                        O(wo[t][oi])
                    oi += 1
                    continue
                g = t - int(tok[1:])
                if not 0 <= g < ng:
                    continue
                if tok[0] in "qkv":
                    out.extend(("P", hd, "qkv".index(tok[0])) for hd in groups[g])
                else:
                    out.append((tok[0], g))
        O(sum(len(g) for g in groups))
        out.extend(("O", h, 1, "x") for h in sp)
        return out
    return f


def build(cfg):
    cfg = dict(cfg)
    cfg["prog"] = prog(**cfg.get("p", {}))

    def fn(A_x, A_mem0, A_Wq, A_Wk, A_Wv, A_Wo, A_seg_len, B_x, B_w_r, B_w_gate, B_w_up, B_w_down):
        B, S, D = A_x.shape
        _, H, Dh = A_Wq.shape
        M = A_mem0.shape[1]
        F = B_w_gate.shape[1]
        SEG = int(A_seg_len)
        NSEG = S // SEG
        L = M + SEG
        anyspec = pl.BlockSpec(memory_space=pl.ANY)
        vspec = pl.BlockSpec(memory_space=pltpu.VMEM)
        out = pl.pallas_call(
            functools.partial(_kernel, S=S, D=D, H=H, Dh=Dh, M=M, SEG=SEG, F=F, cfg=cfg),
            out_shape=jax.ShapeDtypeStruct((S, D), BF16),
            in_specs=[anyspec] * 10,
            out_specs=anyspec,
            scratch_shapes=[
                pltpu.VMEM((M, D), BF16), pltpu.VMEM((D,), BF16),
                pltpu.VMEM((NSEG, 8, D), BF16),
                pltpu.VMEM((NSEG * 8 // 2, D), U32),
                pltpu.VMEM((NSEG, SEG, D), BF16),
                pltpu.VMEM((3 * H // 2, D, Dh), U32),
                pltpu.VMEM((3 * H, D // 2, Dh), U32),
                pltpu.VMEM((NSEG + 2, 3 * H * 8 + SEG * D // LANES, Dh), F32),
                pltpu.VMEM((D // LANES, H * Dh // 2, LANES), U32),
                pltpu.VMEM((D, F), BF16), pltpu.VMEM((D, F), BF16), pltpu.VMEM((F, D), BF16),
                pltpu.VMEM((S, D), F32), pltpu.VMEM((S, D), F32),
                pltpu.VMEM((SEG, D), F32), pltpu.VMEM((2, SEG, LANES), jnp.int32),
                pltpu.VMEM((3 * L, LANES), F32),
                pltpu.VMEM((S, D), BF16),
                pltpu.SemaphoreType.DMA((3 * H // 2,)),
                pltpu.SemaphoreType.DMA((20,)),
            ],
            compiler_params=pltpu.CompilerParams(vmem_limit_bytes=100 * 1024 * 1024, flags=cfg.get("flags")),
            name="rmt",
        )(A_x.reshape(NSEG, SEG, D), A_mem0.reshape(M, D), A_Wq, A_Wk, A_Wv, A_Wo.reshape(H * Dh, D),
          B_w_r, B_w_gate, B_w_up, B_w_down)
        return out.reshape(B, S, D)
    return fn


@functools.partial(jax.jit, static_argnames=("A_seg_len",))
def pallas_sequential_preLN__memory_aug_recurrent_mem_tr__moe_arch_mod__prompt_kernel(
        A_x, A_mem0, A_Wq, A_Wk, A_Wv, A_Wo, A_seg_len, B_x, B_w_r, B_w_gate, B_w_up, B_w_down):
    return build({'UN':4,'p':{'pat': 'q0 k0 O S1 v1 O V3', 'wo': {5: (2, 3), 6: (4, 4), 7: (6, 6), 8: (8, 8), 9: (10, 10), 10: (12, 13), 11: (20, 20), 12: (24, 24), 13: (26, 26)}, 'postat': [5, 6, 7], 'lnat': [3, 4, 5], 'wc': 1, 'split': [20, 24, 28]}})(A_x, A_mem0, A_Wq, A_Wk, A_Wv, A_Wo, A_seg_len, B_x, B_w_r, B_w_gate, B_w_up, B_w_down)
```

```python
import functools
import math

import jax
import jax.numpy as jnp
import numpy as np
from jax import lax
import jax.experimental.pallas as pl
import jax.experimental.pallas.tpu as pltpu

F32 = jnp.float32
BF16 = jnp.bfloat16
U32 = jnp.uint32
I32 = jnp.int32

LANES = 128
AHEAD = 8
PHASES = ((1, 4), (3, 4))
UNROLL = 8
LN_EPS = float(np.asarray(1e-5, dtype=BF16))
KEY_BASE = 0x20000001

WO_UPTO = {5: (2, 3), 6: (4, 4), 7: (6, 6), 8: (8, 8), 9: (10, 10), 10: (12, 13), 11: (20, 21),
           12: (24, 24), 13: (26, 27)}
NEXT_LN_SLOTS = (3, 4, 5)
RESIDUAL_SLOTS = (5, 6, 7, 8)
DEFERRED_HEADS = (20, 24, 28)


def _rb(v):
    return v.astype(BF16).astype(F32)


def _mm(a, b):
    return jnp.dot(a, b, preferred_element_type=F32)


def _layernorm(v):
    n = v.shape[-1]
    mean = jnp.sum(v, axis=-1, keepdims=True) * (1.0 / n)
    yield
    c = v - mean
    var = jnp.sum(c * c, axis=-1, keepdims=True) * (1.0 / n)
    yield
    den = _rb(jnp.sqrt(_rb(_rb(var) + LN_EPS)))
    return _rb(_rb(v - _rb(mean)) / den)


def _finish(stages):
    while True:
        try:
            next(stages)
        except StopIteration as stop:
            return stop.value


def _kernel(x_hbm, mem0_hbm, wq_hbm, wk_hbm, wv_hbm, wo_hbm, wr_hbm, wg_hbm, wu_hbm, wd_hbm,
            out_hbm,
            mem0_v, wr_v, xa_v, xan_v, x_v, raw_v, w_v, pre_v, wo_v, wg_v, wu_v, wd_v,
            h_v, hn_v, att_v, cap_v, out_v, wsem, sems):
    NSEG, SEG, D = x_hbm.shape
    _, H, Dh = wq_hbm.shape
    M = mem0_hbm.shape[0]
    S = NSEG * SEG
    L = M + SEG
    G = LANES // L
    NCOL = D // LANES
    XN = 3 * H * AHEAD
    scale = Dh ** -0.5

    free_sems = iter(range(sems.shape[0]))

    def new_copy(src, dst):
        return pltpu.make_async_copy(src, dst, sems.at[next(free_sems)])

    half = NSEG // 2
    cp_xa = new_copy(x_hbm.at[:, pl.ds(0, AHEAD), :], xa_v)
    cp_loop = [new_copy(mem0_hbm, mem0_v), new_copy(wr_hbm, wr_v)]
    cp_loop += [new_copy(x_hbm.at[pl.ds(a, half)], x_v.at[pl.ds(a, half)]) for a in (0, half)]
    cp_loop += [new_copy(wo_hbm.at[:, pl.ds(n * LANES, LANES)], wo_v.bitcast(BF16).at[n])
                for n in range(NCOL)]
    cp_ffn = [new_copy(wg_hbm, wg_v), new_copy(wu_hbm, wu_v), new_copy(wd_hbm, wd_v)]

    def start_weights(first, last):
        for k in range(first, last):
            j, m = divmod(k, 3)
            src = (wq_hbm, wk_hbm, wv_hbm)[m].bitcast(U32).at[:, j, :]
            pltpu.make_async_copy(src, raw_v.at[k], wsem.at[k]).start()

    cp_xa.start()
    start_weights(0, 1)

    ri = lax.broadcasted_iota(I32, (L, LANES), 0)
    ci = lax.broadcasted_iota(I32, (L, LANES), 1)
    for g in range(G):
        cj = ci - g * L
        own = (cj >= 0) & (cj < L)
        keep = own & ((ri < M) | (ri >= cj))
        fill = jnp.where(own, -1e9 / scale, -jnp.inf)
        cap_v[pl.ds(g * L, L), :] = jnp.where(keep, 1.0, fill).astype(F32)

    top = [pre_v.at[NSEG, pl.ds(i * SEG, SEG), :] for i in range(2)]
    for t in top:
        t[...] = jnp.zeros((SEG, LANES), F32)
    att_v[...] = jnp.zeros((SEG, D), F32)

    cp_xa.wait()
    start_weights(1, 3)

    def ln_ahead(i, carry):
        v = xa_v[pl.ds(pl.multiple_of(i * half, half), half)].astype(F32).reshape(half * AHEAD, D)
        rows = half * AHEAD // 2
        xan_v[pl.ds(pl.multiple_of(i * rows, rows), rows), :] = pltpu.bitcast(
            _finish(_layernorm(v)).astype(BF16), U32)
        return carry

    lax.fori_loop(0, 2, ln_ahead, 0)

    bounds = [0]
    for pairs, iters in PHASES:
        bounds += [bounds[-1] + pairs * (c + 1) for c in range(iters)]
    n_iter = len(bounds) - 1
    assert bounds[-1] == H // 2 and bounds[1] == 1

    def prefetch(g):
        first = bounds[min(g + 2, n_iter)] if g > 1 else bounds[g + 1]
        last = bounds[min(g + 3, n_iter)] if g > 0 else bounds[2]
        start_weights(3 * first, 3 * last)
        for n, cp in enumerate(cp_loop):
            if 3 + n * (n_iter - 4) // len(cp_loop) == g:
                cp.start()

    def project_ahead(g0, pairs, iters, i, carry):
        j0 = bounds[g0] + i * pairs
        for u in range(3 * pairs):
            k = 3 * j0 + u
            pltpu.make_async_copy(raw_v.at[k], raw_v.at[k], wsem.at[k]).wait()
        for c in range(iters):
            pl.when(i == c)(functools.partial(prefetch, g0 + c))
        for u in range(pairs):
            for m in range(3):
                j = j0 + u
                w = raw_v[3 * j + m]
                even = pltpu.bitcast(w << 16, F32).astype(BF16)
                odd = pltpu.bitcast(w & np.uint32(0xFFFF0000), F32).astype(BF16)
                for t, wt in enumerate((even, odd)):
                    hm = (2 * j + t) * 3 + m
                    w_v[hm] = pltpu.bitcast(wt, U32)
                    d = _mm(pltpu.bitcast(xan_v[...], BF16), wt)
                    pre_v[pl.ds(0, NSEG), pl.ds(pl.multiple_of(hm * AHEAD, AHEAD), AHEAD), :] = (
                        d.reshape(NSEG, AHEAD, Dh))
        return carry

    g0 = 0
    for pairs, iters in PHASES:
        lax.fori_loop(0, iters, functools.partial(project_ahead, g0, pairs, iters), 0)
        g0 += iters
    for cp in cp_loop:
        cp.wait()
    for cp in cp_ffn:
        cp.start()

    def ln_segment(s):
        v = yield from _layernorm(x_v[s].astype(F32))
        for n in range(NCOL):
            pre_v[s, pl.ds(XN + n * SEG, SEG), :] = v[:, n * LANES:(n + 1) * LANES]

    _finish(ln_segment(0))
    wr = wr_v[...].astype(F32).reshape(1, D)
    row_id = lax.broadcasted_iota(I32, (SEG, LANES), 0)

    def residual(s, live):
        r0 = pl.multiple_of(s * SEG, SEG)
        h = _rb(x_v[s].astype(F32) + _rb(att_v[...]))
        h_v[pl.ds(r0, SEG), :] = h
        hn = yield from _layernorm(h)
        hn_v[pl.ds(r0, SEG), :] = hn
        out_v[pl.ds(r0, SEG), :] = (h + hn).astype(BF16)
        r = jnp.broadcast_to(_rb(jnp.sum(hn * wr, axis=-1, keepdims=True)), (SEG, LANES))
        u = pltpu.bitcast(r, I32) >> 16
        rank = jnp.where(r == r, (u ^ ((u >> 15) & 0x7FFF)) + 0x8000, 0)
        key = jnp.where(live, rank * S + (S - 1 - r0) - row_id, -1)
        key = pltpu.bitcast(key + KEY_BASE, F32)
        yield
        best = top[0][...]
        top[0][...] = jnp.maximum(best, key)
        top[1][...] = jnp.maximum(top[1][...], jnp.minimum(best, key))

    groups = [range(a, min(a + G, H)) for a in range(0, H, G)]
    exp2_scale = scale * math.log2(math.e)

    def step(s, mem, deferred):
        xs = jnp.concatenate([pre_v[s, pl.ds(XN + n * SEG, SEG), :] for n in range(NCOL)], axis=1)
        lhs = jnp.concatenate([xs[AHEAD:], mem], axis=0).astype(BF16)
        qkv, probs, heads = {}, {}, {}
        acc_mem, acc_x = [None] * NCOL, [None] * NCOL
        next_ln = ln_segment(jnp.minimum(s + 1, NSEG - 1))
        prev = residual(jnp.maximum(s - 1, 0), s > 0)

        def project(g, m):
            for hd in groups[g]:
                d = _mm(lhs, pltpu.bitcast(w_v[hd * 3 + m], BF16))
                early = pre_v[s, pl.ds((hd * 3 + m) * AHEAD, AHEAD), :]
                qkv[hd, m] = jnp.concatenate([d[SEG - AHEAD:], early, d[:SEG - AHEAD]], axis=0)

        def stacked(g, m):
            return [qkv.pop((hd, m)) for hd in groups[g]]

        def tile(g, m):
            pad = jnp.zeros((LANES - len(groups[g]) * L, Dh), F32)
            return jnp.concatenate(stacked(g, m) + [pad], axis=0).astype(BF16)

        def scores(g):
            q = jnp.concatenate(stacked(g, 0), axis=0)
            sc = lax.dot_general(q, tile(g, 1), (((1,), (1,)), ((), ())), preferred_element_type=F32)
            cap = cap_v[pl.ds(0, q.shape[0]), :]
            sc = jnp.where(cap > 0.0, sc, cap)
            probs[g] = jnp.exp2((sc - jnp.max(sc, axis=-1, keepdims=True)) * exp2_scale)

        def attend(g):
            v = tile(g, 2)
            e = probs.pop(g)
            inv = pltpu.reciprocal(jnp.sum(e, axis=-1, keepdims=True), full_range=False)
            o = _mm(e, v) * inv
            for i, hd in enumerate(groups[g]):
                heads[hd] = o[i * L:(i + 1) * L]

        def output(hd, with_mem, with_x):
            o = heads[hd][(0 if with_mem else M):(L if with_x else M)]
            for n in range(NCOL):
                d = _mm(o, pltpu.bitcast(wo_v[n, pl.ds(hd * Dh // 2, Dh // 2), :], BF16))
                if with_mem:
                    acc_mem[n] = d[:M] if acc_mem[n] is None else acc_mem[n] + d[:M]
                if with_x:
                    acc_x[n] = d[-SEG:] if acc_x[n] is None else acc_x[n] + d[-SEG:]

        pending = list(range(H))

        def output_upto(end):
            while pending and pending[0] < end:
                hd = pending.pop(0)
                output(hd, True, hd not in deferred)

        ng = len(groups)
        for t in range(ng + 3):
            if t in RESIDUAL_SLOTS:
                next(prev, None)
            if t in NEXT_LN_SLOTS:
                next(next_ln, None)
            if t < ng:
                project(t, 0)
                project(t, 1)
            output_upto(WO_UPTO.get(t, (0, 0))[0])
            if 0 <= t - 1 < ng:
                scores(t - 1)
                project(t - 1, 2)
            output_upto(WO_UPTO.get(t, (0, 0))[1])
            if t >= 3:
                attend(t - 3)
        output_upto(H)
        for hd in deferred:
            output(hd, False, True)
        _finish(prev)
        _finish(next_ln)
        att_v[...] = jnp.concatenate(acc_x, axis=1)
        return jnp.concatenate(acc_mem, axis=1)

    flush_at = NSEG // UNROLL - 1
    done = (flush_at * UNROLL - 1) * SEG
    cp_head = new_copy(out_v.at[pl.ds(0, done)], out_hbm.at[pl.ds(0, done)])
    cp_tail = new_copy(out_v.at[pl.ds(done, S - done)], out_hbm.at[pl.ds(done, S - done)])

    def steps(i, mem):
        pl.when(i == flush_at)(cp_head.start)
        for u in range(UNROLL):
            mem = step(i * UNROLL + u, mem, DEFERRED_HEADS if u < UNROLL - 1 else ())
        return mem

    lax.fori_loop(0, NSEG // UNROLL, steps, mem0_v[...].astype(F32))

    for cp in cp_ffn:
        cp.wait()
    _finish(residual(NSEG - 1, True))
    cp_tail.start()

    best = top[0][...]
    k1 = jnp.max(best, axis=0, keepdims=True)
    k2 = jnp.max(jnp.where(best == k1, top[1][...], best), axis=0, keepdims=True)
    i1, i2 = [
        S - 1 - lax.rem((pltpu.bitcast(jnp.broadcast_to(k, (8, LANES)), I32) - KEY_BASE)[0, 0], S)
        for k in (k1, k2)]
    first = lax.broadcasted_iota(I32, (8, D), 0) == 0
    h_sel = jnp.where(first, h_v[pl.ds(i1, 1), :], h_v[pl.ds(i2, 1), :])
    x_sel = jnp.where(first, hn_v[pl.ds(i1, 1), :], hn_v[pl.ds(i2, 1), :])
    gate = _rb(_mm(x_sel, wg_v[...]))
    up = _rb(_mm(x_sel, wu_v[...]))
    y = _rb(_mm(_rb(_rb(gate * jax.nn.sigmoid(gate)) * up), wd_v[...]))
    r_sel = _rb(jnp.sum(x_sel * wr, axis=-1, keepdims=True))
    routed = h_sel + _rb(x_sel + _rb(y * _rb(jax.nn.sigmoid(r_sel))))

    cp_head.wait()
    cp_tail.wait()
    row16 = lax.broadcasted_iota(I32, (16, D), 0)
    blocks = []
    for j, idx in enumerate((i1, i2)):
        b0 = pl.multiple_of((idx // 16) * 16, 16)
        cur = out_v[pl.ds(b0, 16), :].astype(F32)
        out_v[pl.ds(b0, 16), :] = jnp.where(row16 == idx - b0, routed[j:j + 1], cur).astype(BF16)
        blocks.append(b0)
    patch = [new_copy(out_v.at[pl.ds(b0, 16)], out_hbm.at[pl.ds(b0, 16)]) for b0 in blocks]
    patch[0].start()

    @pl.when(blocks[0] != blocks[1])
    def _():
        patch[1].start()
        patch[1].wait()

    patch[0].wait()


@functools.partial(jax.jit, static_argnames=("A_seg_len",))
def pallas_sequential_preLN__memory_aug_recurrent_mem_tr__moe_arch_mod__prompt_kernel(
    A_x: jax.Array,
    A_mem0: jax.Array,
    A_Wq: jax.Array,
    A_Wk: jax.Array,
    A_Wv: jax.Array,
    A_Wo: jax.Array,
    A_seg_len: int,
    B_x: jax.Array,
    B_w_r: jax.Array,
    B_w_gate: jax.Array,
    B_w_up: jax.Array,
    B_w_down: jax.Array,
):
    del B_x
    B, S, D = A_x.shape
    _, H, Dh = A_Wq.shape
    M = A_mem0.shape[1]
    F = B_w_gate.shape[1]
    SEG = A_seg_len
    NSEG = S // SEG
    L = M + SEG
    assert B == 1 and Dh == LANES and NSEG % UNROLL == 0

    hbm = pl.BlockSpec(memory_space=pl.ANY)
    out = pl.pallas_call(
        _kernel,
        out_shape=jax.ShapeDtypeStruct((S, D), BF16),
        in_specs=[hbm] * 10,
        out_specs=hbm,
        scratch_shapes=[
            pltpu.VMEM((M, D), BF16),
            pltpu.VMEM((D,), BF16),
            pltpu.VMEM((NSEG, AHEAD, D), BF16),
            pltpu.VMEM((NSEG * AHEAD // 2, D), U32),
            pltpu.VMEM((NSEG, SEG, D), BF16),
            pltpu.VMEM((3 * H // 2, D, Dh), U32),
            pltpu.VMEM((3 * H, D // 2, Dh), U32),
            pltpu.VMEM((NSEG + 1, 3 * H * AHEAD + SEG * D // LANES, Dh), F32),
            pltpu.VMEM((D // LANES, H * Dh // 2, LANES), U32),
            pltpu.VMEM((D, F), BF16),
            pltpu.VMEM((D, F), BF16),
            pltpu.VMEM((F, D), BF16),
            pltpu.VMEM((S, D), F32),
            pltpu.VMEM((S, D), F32),
            pltpu.VMEM((SEG, D), F32),
            pltpu.VMEM((LANES // L * L, LANES), F32),
            pltpu.VMEM((S, D), BF16),
            pltpu.SemaphoreType.DMA((3 * H // 2,)),
            pltpu.SemaphoreType.DMA((12 + D // LANES,)),
        ],
        compiler_params=pltpu.CompilerParams(vmem_limit_bytes=100 * 1024 * 1024),
        name="rmt_mod",
    )(A_x.reshape(NSEG, SEG, D), A_mem0.reshape(M, D), A_Wq, A_Wk, A_Wv, A_Wo.reshape(H * Dh, D),
      B_w_r, B_w_gate, B_w_up, B_w_down)
    return out.reshape(B, S, D)
```

```python
import functools
import math

import jax
import jax.numpy as jnp
import numpy as np
from jax import lax
import jax.experimental.pallas as pl
import jax.experimental.pallas.tpu as pltpu

F32 = jnp.float32
BF16 = jnp.bfloat16
U32 = jnp.uint32
I32 = jnp.int32

LANES = 128
AHEAD = 8
PHASES = ((1, 4), (3, 4))
UNROLL = 8
LN_EPS = float(np.asarray(1e-5, dtype=BF16))
KEY_BASE = 0x20000001

WO_UPTO = {5: (2, 3), 6: (4, 4), 7: (6, 6), 8: (8, 8), 9: (10, 10), 10: (12, 13), 11: (20, 21),
           12: (24, 24), 13: (26, 27)}
NEXT_LN_SLOTS = (3, 4, 5)
RESIDUAL_SLOTS = (5, 6, 7, 8)
DEFERRED_HEADS = (20, 24, 28)


def _rb(v):
    return v.astype(BF16).astype(F32)


def _mm(a, b):
    return jnp.dot(a, b, preferred_element_type=F32)


def _layernorm(v):
    n = v.shape[-1]
    mean = jnp.sum(v, axis=-1, keepdims=True) * (1.0 / n)
    yield
    c = v - mean
    var = jnp.sum(c * c, axis=-1, keepdims=True) * (1.0 / n)
    yield
    den = _rb(jnp.sqrt(_rb(_rb(var) + LN_EPS)))
    return _rb(_rb(v - _rb(mean)) / den)


def _finish(stages):
    while True:
        try:
            next(stages)
        except StopIteration as stop:
            return stop.value


def _kernel(x_hbm, mem0_hbm, wq_hbm, wk_hbm, wv_hbm, wo_hbm, wr_hbm, wg_hbm, wu_hbm, wd_hbm,
            out_hbm,
            mem0_v, wr_v, xa_v, xan_v, x_v, raw_v, w_v, pre_v, wo_v, wg_v, wu_v, wd_v,
            h_v, hn_v, att_v, cap_v, out_v, wsem, sems):
    NSEG, SEG, D = x_hbm.shape
    _, H, Dh = wq_hbm.shape
    M = mem0_hbm.shape[0]
    S = NSEG * SEG
    L = M + SEG
    G = LANES // L
    NCOL = D // LANES
    XN = 3 * H * AHEAD
    scale = Dh ** -0.5

    free_sems = iter(range(sems.shape[0]))

    def new_copy(src, dst):
        return pltpu.make_async_copy(src, dst, sems.at[next(free_sems)])

    half = NSEG // 2
    cp_xa = new_copy(x_hbm.at[:, pl.ds(0, AHEAD), :], xa_v)
    cp_loop = [new_copy(mem0_hbm, mem0_v), new_copy(wr_hbm, wr_v)]
    cp_loop += [new_copy(x_hbm.at[pl.ds(a, half)], x_v.at[pl.ds(a, half)]) for a in (0, half)]
    cp_loop += [new_copy(wo_hbm.bitcast(U32).at[:, pl.ds(n * LANES, LANES)], wo_v.at[n])
                for n in range(NCOL)]
    cp_ffn = [new_copy(wg_hbm, wg_v), new_copy(wu_hbm, wu_v), new_copy(wd_hbm, wd_v)]

    def start_weights(first, last):
        for k in range(first, last):
            j, m = divmod(k, 3)
            src = (wq_hbm, wk_hbm, wv_hbm)[m].bitcast(U32).at[:, j, :]
            pltpu.make_async_copy(src, raw_v.at[k], wsem.at[k]).start()

    cp_xa.start()
    start_weights(0, 1)

    ri = lax.broadcasted_iota(I32, (L, LANES), 0)
    ci = lax.broadcasted_iota(I32, (L, LANES), 1)
    for g in range(G):
        cj = ci - g * L
        own = (cj >= 0) & (cj < L)
        keep = own & ((ri < M) | (ri >= cj))
        fill = jnp.where(own, -1e9 / scale, -jnp.inf)
        cap_v[pl.ds(g * L, L), :] = jnp.where(keep, 1.0, fill).astype(F32)

    top = [pre_v.at[NSEG, pl.ds(i * SEG, SEG), :] for i in range(2)]
    for t in top:
        t[...] = jnp.zeros((SEG, LANES), F32)
    att_v[...] = jnp.zeros((SEG, D), F32)

    cp_xa.wait()
    start_weights(1, 3)

    def ln_ahead(i, carry):
        v = xa_v[pl.ds(pl.multiple_of(i * half, half), half)].astype(F32).reshape(half * AHEAD, D)
        rows = half * AHEAD // 2
        xan_v[pl.ds(pl.multiple_of(i * rows, rows), rows), :] = pltpu.bitcast(
            _finish(_layernorm(v)).astype(BF16), U32)
        return carry

    lax.fori_loop(0, 2, ln_ahead, 0)

    bounds = [0]
    for pairs, iters in PHASES:
        bounds += [bounds[-1] + pairs * (c + 1) for c in range(iters)]
    n_iter = len(bounds) - 1
    assert bounds[-1] == H // 2 and bounds[1] == 1

    def prefetch(g):
        first = bounds[min(g + 2, n_iter)] if g > 1 else bounds[g + 1]
        last = bounds[min(g + 3, n_iter)] if g > 0 else bounds[2]
        start_weights(3 * first, 3 * last)
        for n, cp in enumerate(cp_loop):
            if 3 + n * (n_iter - 4) // len(cp_loop) == g:
                cp.start()

    def project_ahead(g0, pairs, iters, i, carry):
        j0 = bounds[g0] + i * pairs
        for u in range(3 * pairs):
            k = 3 * j0 + u
            pltpu.make_async_copy(raw_v.at[k], raw_v.at[k], wsem.at[k]).wait()
        for c in range(iters):
            pl.when(i == c)(functools.partial(prefetch, g0 + c))
        for u in range(pairs):
            for m in range(3):
                j = j0 + u
                w = raw_v[3 * j + m]
                even = pltpu.bitcast(w << 16, F32).astype(BF16)
                odd = pltpu.bitcast(w & np.uint32(0xFFFF0000), F32).astype(BF16)
                for t, wt in enumerate((even, odd)):
                    hm = (2 * j + t) * 3 + m
                    w_v[hm] = pltpu.bitcast(wt, U32)
                    d = _mm(pltpu.bitcast(xan_v[...], BF16), wt)
                    pre_v[pl.ds(0, NSEG), pl.ds(pl.multiple_of(hm * AHEAD, AHEAD), AHEAD), :] = (
                        d.reshape(NSEG, AHEAD, Dh))
        return carry

    g0 = 0
    for pairs, iters in PHASES:
        lax.fori_loop(0, iters, functools.partial(project_ahead, g0, pairs, iters), 0)
        g0 += iters
    for cp in cp_loop:
        cp.wait()
    for cp in cp_ffn:
        cp.start()

    def ln_segment(s):
        v = yield from _layernorm(x_v[s].astype(F32))
        for n in range(NCOL):
            pre_v[s, pl.ds(XN + n * SEG, SEG), :] = v[:, n * LANES:(n + 1) * LANES]

    _finish(ln_segment(0))
    wr = wr_v[...].astype(F32).reshape(1, D)
    row_id = lax.broadcasted_iota(I32, (SEG, LANES), 0)

    def residual(s, live):
        r0 = pl.multiple_of(s * SEG, SEG)
        h = _rb(x_v[s].astype(F32) + _rb(att_v[...]))
        h_v[pl.ds(r0, SEG), :] = h
        hn = yield from _layernorm(h)
        hn_v[pl.ds(r0, SEG), :] = hn
        out_v[pl.ds(r0, SEG), :] = (h + hn).astype(BF16)
        r = jnp.broadcast_to(_rb(jnp.sum(hn * wr, axis=-1, keepdims=True)), (SEG, LANES))
        u = pltpu.bitcast(r, I32) >> 16
        rank = jnp.where(r == r, (u ^ ((u >> 15) & 0x7FFF)) + 0x8000, 0)
        key = jnp.where(live, rank * S + (S - 1 - r0) - row_id, -1)
        key = pltpu.bitcast(key + KEY_BASE, F32)
        yield
        best = top[0][...]
        top[0][...] = jnp.maximum(best, key)
        top[1][...] = jnp.maximum(top[1][...], jnp.minimum(best, key))

    groups = [range(a, min(a + G, H)) for a in range(0, H, G)]
    exp2_scale = scale * math.log2(math.e)

    def step(s, mem, deferred):
        xs = jnp.concatenate([pre_v[s, pl.ds(XN + n * SEG, SEG), :] for n in range(NCOL)], axis=1)
        lhs = jnp.concatenate([xs[AHEAD:], mem], axis=0).astype(BF16)
        qkv, probs, heads = {}, {}, {}
        acc_mem, acc_x = [None] * NCOL, [None] * NCOL
        next_ln = ln_segment(jnp.minimum(s + 1, NSEG - 1))
        prev = residual(jnp.maximum(s - 1, 0), s > 0)

        def project(g, m):
            for hd in groups[g]:
                d = _mm(lhs, pltpu.bitcast(w_v[hd * 3 + m], BF16))
                early = pre_v[s, pl.ds((hd * 3 + m) * AHEAD, AHEAD), :]
                qkv[hd, m] = jnp.concatenate([d[SEG - AHEAD:], early, d[:SEG - AHEAD]], axis=0)

        def stacked(g, m):
            return [qkv.pop((hd, m)) for hd in groups[g]]

        def tile(g, m):
            pad = jnp.zeros((LANES - len(groups[g]) * L, Dh), F32)
            return jnp.concatenate(stacked(g, m) + [pad], axis=0).astype(BF16)

        def scores(g):
            q = jnp.concatenate(stacked(g, 0), axis=0)
            sc = lax.dot_general(q, tile(g, 1), (((1,), (1,)), ((), ())), preferred_element_type=F32)
            cap = cap_v[pl.ds(0, q.shape[0]), :]
            sc = jnp.where(cap > 0.0, sc, cap)
            probs[g] = jnp.exp2((sc - jnp.max(sc, axis=-1, keepdims=True)) * exp2_scale)

        def attend(g):
            v = tile(g, 2)
            e = probs.pop(g)
            inv = pltpu.reciprocal(jnp.sum(e, axis=-1, keepdims=True), full_range=False)
            o = _mm(e, v) * inv
            for i, hd in enumerate(groups[g]):
                heads[hd] = o[i * L:(i + 1) * L]

        def output(hd, with_mem, with_x):
            o = heads[hd][(0 if with_mem else M):(L if with_x else M)]
            for n in range(NCOL):
                d = _mm(o, pltpu.bitcast(wo_v[n, pl.ds(hd * Dh // 2, Dh // 2), :], BF16))
                if with_mem:
                    acc_mem[n] = d[:M] if acc_mem[n] is None else acc_mem[n] + d[:M]
                if with_x:
                    acc_x[n] = d[-SEG:] if acc_x[n] is None else acc_x[n] + d[-SEG:]

        pending = list(range(H))

        def output_upto(end):
            while pending and pending[0] < end:
                hd = pending.pop(0)
                output(hd, True, hd not in deferred)

        ng = len(groups)
        for t in range(ng + 3):
            if t in RESIDUAL_SLOTS:
                next(prev, None)
            if t in NEXT_LN_SLOTS:
                next(next_ln, None)
            if t < ng:
                project(t, 0)
                project(t, 1)
            output_upto(WO_UPTO.get(t, (0, 0))[0])
            if 0 <= t - 1 < ng:
                scores(t - 1)
                project(t - 1, 2)
            output_upto(WO_UPTO.get(t, (0, 0))[1])
            if t >= 3:
                attend(t - 3)
        output_upto(H)
        for hd in deferred:
            output(hd, False, True)
        _finish(prev)
        _finish(next_ln)
        att_v[...] = jnp.concatenate(acc_x, axis=1)
        return jnp.concatenate(acc_mem, axis=1)

    flush_at = NSEG // UNROLL - 1
    done = (flush_at * UNROLL - 1) * SEG
    cp_head = new_copy(out_v.at[pl.ds(0, done)], out_hbm.at[pl.ds(0, done)])
    cp_tail = new_copy(out_v.at[pl.ds(done, S - done)], out_hbm.at[pl.ds(done, S - done)])

    def steps(i, mem):
        pl.when(i == flush_at)(cp_head.start)
        for u in range(UNROLL):
            mem = step(i * UNROLL + u, mem, DEFERRED_HEADS if u < UNROLL - 1 else ())
        return mem

    lax.fori_loop(0, NSEG // UNROLL, steps, mem0_v[...].astype(F32))

    for cp in cp_ffn:
        cp.wait()
    _finish(residual(NSEG - 1, True))
    cp_tail.start()

    best = top[0][...]
    k1 = jnp.max(best, axis=0, keepdims=True)
    k2 = jnp.max(jnp.where(best == k1, top[1][...], best), axis=0, keepdims=True)

    def token(key):
        key = pltpu.bitcast(jnp.broadcast_to(key, (8, LANES)), I32) - KEY_BASE
        return jnp.clip(S - 1 - lax.rem(key[0, 0], S), 0, S - 1)

    i1, i2 = token(k1), token(k2)
    first = lax.broadcasted_iota(I32, (8, D), 0) == 0
    h_sel = jnp.where(first, h_v[pl.ds(i1, 1), :], h_v[pl.ds(i2, 1), :])
    x_sel = jnp.where(first, hn_v[pl.ds(i1, 1), :], hn_v[pl.ds(i2, 1), :])
    gate = _rb(_mm(x_sel, wg_v[...]))
    up = _rb(_mm(x_sel, wu_v[...]))
    y = _rb(_mm(_rb(_rb(gate * jax.nn.sigmoid(gate)) * up), wd_v[...]))
    r_sel = _rb(jnp.sum(x_sel * wr, axis=-1, keepdims=True))
    routed = h_sel + _rb(x_sel + _rb(y * _rb(jax.nn.sigmoid(r_sel))))

    cp_head.wait()
    cp_tail.wait()
    row16 = lax.broadcasted_iota(I32, (16, D), 0)
    blocks = []
    for j, idx in enumerate((i1, i2)):
        b0 = pl.multiple_of((idx // 16) * 16, 16)
        cur = out_v[pl.ds(b0, 16), :].astype(F32)
        out_v[pl.ds(b0, 16), :] = jnp.where(row16 == idx - b0, routed[j:j + 1], cur).astype(BF16)
        blocks.append(b0)
    patch = [new_copy(out_v.at[pl.ds(b0, 16)], out_hbm.at[pl.ds(b0, 16)]) for b0 in blocks]
    patch[0].start()

    @pl.when(blocks[0] != blocks[1])
    def _():
        patch[1].start()
        patch[1].wait()

    patch[0].wait()


@functools.partial(jax.jit, static_argnames=("A_seg_len",))
def pallas_sequential_preLN__memory_aug_recurrent_mem_tr__moe_arch_mod__prompt_kernel(
    A_x: jax.Array,
    A_mem0: jax.Array,
    A_Wq: jax.Array,
    A_Wk: jax.Array,
    A_Wv: jax.Array,
    A_Wo: jax.Array,
    A_seg_len: int,
    B_x: jax.Array,
    B_w_r: jax.Array,
    B_w_gate: jax.Array,
    B_w_up: jax.Array,
    B_w_down: jax.Array,
):
    del B_x
    B, S, D = A_x.shape
    _, H, Dh = A_Wq.shape
    M = A_mem0.shape[1]
    F = B_w_gate.shape[1]
    SEG = A_seg_len
    NSEG = S // SEG
    L = M + SEG
    assert B == 1 and Dh == LANES and NSEG % UNROLL == 0

    hbm = pl.BlockSpec(memory_space=pl.ANY)
    out = pl.pallas_call(
        _kernel,
        out_shape=jax.ShapeDtypeStruct((S, D), BF16),
        in_specs=[hbm] * 10,
        out_specs=hbm,
        scratch_shapes=[
            pltpu.VMEM((M, D), BF16),
            pltpu.VMEM((D,), BF16),
            pltpu.VMEM((NSEG, AHEAD, D), BF16),
            pltpu.VMEM((NSEG * AHEAD // 2, D), U32),
            pltpu.VMEM((NSEG, SEG, D), BF16),
            pltpu.VMEM((3 * H // 2, D, Dh), U32),
            pltpu.VMEM((3 * H, D // 2, Dh), U32),
            pltpu.VMEM((NSEG + 1, 3 * H * AHEAD + SEG * D // LANES, Dh), F32),
            pltpu.VMEM((D // LANES, H * Dh // 2, LANES), U32),
            pltpu.VMEM((D, F), BF16),
            pltpu.VMEM((D, F), BF16),
            pltpu.VMEM((F, D), BF16),
            pltpu.VMEM((S, D), F32),
            pltpu.VMEM((S, D), F32),
            pltpu.VMEM((SEG, D), F32),
            pltpu.VMEM((LANES // L * L, LANES), F32),
            pltpu.VMEM((S, D), BF16),
            pltpu.SemaphoreType.DMA((3 * H // 2,)),
            pltpu.SemaphoreType.DMA((12 + D // LANES,)),
        ],
        compiler_params=pltpu.CompilerParams(vmem_limit_bytes=100 * 1024 * 1024),
        name="rmt_mod",
    )(A_x.reshape(NSEG, SEG, D), A_mem0.reshape(M, D), A_Wq, A_Wk, A_Wv, A_Wo.reshape(H * Dh, D),
      B_w_r, B_w_gate, B_w_up, B_w_down)
    return out.reshape(B, S, D)
```

```python
import functools
import math

import jax
import jax.numpy as jnp
import numpy as np
from jax import lax
import jax.experimental.pallas as pl
import jax.experimental.pallas.tpu as pltpu

F32 = jnp.float32
BF16 = jnp.bfloat16
U32 = jnp.uint32
I32 = jnp.int32

LANES = 128
AHEAD = 8
PHASES = ((1, 4), (3, 4))
UNROLL = 8
LN_EPS = float(np.asarray(1e-5, dtype=BF16))
KEY_BASE = 0x20000001

WO_UPTO = {5: (2, 2), 6: (4, 4), 7: (5, 6), 8: (8, 8), 9: (9, 10), 10: (11, 13), 11: (20, 21),
           12: (21, 24), 13: (24, 27)}
NEXT_LN_SLOTS = (3, 4, 5)
RESIDUAL_SLOTS = (4, 6, 8, 9)
DEFERRED_HEADS = (20, 23, 28)


def _rb(v):
    return v.astype(BF16).astype(F32)


def _mm(a, b):
    return jnp.dot(a, b, preferred_element_type=F32)


def _sigmoid(v):
    return _rb(1.0 / _rb(1.0 + _rb(jnp.exp(-v))))


def _layernorm(v):
    n = v.shape[-1]
    mean = jnp.sum(v, axis=-1, keepdims=True) * (1.0 / n)
    yield
    c = v - mean
    var = jnp.sum(c * c, axis=-1, keepdims=True) * (1.0 / n)
    yield
    den = _rb(jnp.sqrt(_rb(_rb(var) + LN_EPS)))
    return _rb(_rb(v - _rb(mean)) / den)


def _finish(stages):
    while True:
        try:
            next(stages)
        except StopIteration as stop:
            return stop.value


def _kernel(x_hbm, mem0_hbm, wq_hbm, wk_hbm, wv_hbm, wo_hbm, wr_hbm, wg_hbm, wu_hbm, wd_hbm,
            out_hbm,
            mem0_v, wr_v, xa_v, xan_v, x_v, raw_v, w_v, pre_v, wo_v, wg_v, wu_v, wd_v,
            h_v, hn_v, att_v, cap_v, out_v, wsem, sems):
    NSEG, SEG, D = x_hbm.shape
    _, H, Dh = wq_hbm.shape
    M = mem0_hbm.shape[0]
    S = NSEG * SEG
    L = M + SEG
    G = LANES // L
    NCOL = D // LANES
    XN = 3 * H * AHEAD
    scale = Dh ** -0.5

    free_sems = iter(range(sems.shape[0]))

    def new_copy(src, dst):
        return pltpu.make_async_copy(src, dst, sems.at[next(free_sems)])

    half = NSEG // 2
    cp_xa = new_copy(x_hbm.at[:, pl.ds(0, AHEAD), :], xa_v)
    cp_loop = [new_copy(mem0_hbm, mem0_v), new_copy(wr_hbm, wr_v)]
    cp_loop += [new_copy(x_hbm.at[pl.ds(a, half)], x_v.at[pl.ds(a, half)]) for a in (0, half)]
    cp_loop += [new_copy(wo_hbm.bitcast(U32).at[:, pl.ds(n * LANES, LANES)], wo_v.at[n])
                for n in range(NCOL)]
    cp_ffn = [new_copy(wg_hbm, wg_v), new_copy(wu_hbm, wu_v), new_copy(wd_hbm, wd_v)]

    def start_weights(first, last):
        for k in range(first, last):
            j, m = divmod(k, 3)
            src = (wq_hbm, wk_hbm, wv_hbm)[m].bitcast(U32).at[:, j, :]
            pltpu.make_async_copy(src, raw_v.at[k], wsem.at[k]).start()

    cp_xa.start()
    start_weights(0, 1)

    ri = lax.broadcasted_iota(I32, (L, LANES), 0)
    ci = lax.broadcasted_iota(I32, (L, LANES), 1)
    for g in range(G):
        cj = ci - g * L
        own = (cj >= 0) & (cj < L)
        keep = own & ((ri < M) | (ri >= cj))
        fill = jnp.where(own, -1e9 / scale, -jnp.inf)
        cap_v[pl.ds(g * L, L), :] = jnp.where(keep, 1.0, fill).astype(F32)

    top = [pre_v.at[NSEG, pl.ds(i * SEG, SEG), :] for i in range(2)]
    for t in top:
        t[...] = jnp.zeros((SEG, LANES), F32)
    att_v[...] = jnp.zeros((SEG, D), F32)

    cp_xa.wait()
    start_weights(1, 3)

    def ln_ahead(i, carry):
        v = xa_v[pl.ds(pl.multiple_of(i * half, half), half)].astype(F32).reshape(half * AHEAD, D)
        rows = half * AHEAD // 2
        xan_v[pl.ds(pl.multiple_of(i * rows, rows), rows), :] = pltpu.bitcast(
            _finish(_layernorm(v)).astype(BF16), U32)
        return carry

    lax.fori_loop(0, 2, ln_ahead, 0)

    bounds = [0]
    for pairs, iters in PHASES:
        bounds += [bounds[-1] + pairs * (c + 1) for c in range(iters)]
    n_iter = len(bounds) - 1
    assert bounds[-1] == H // 2 and bounds[1] == 1

    def prefetch(g):
        first = bounds[min(g + 2, n_iter)] if g > 1 else bounds[g + 1]
        last = bounds[min(g + 3, n_iter)] if g > 0 else bounds[2]
        start_weights(3 * first, 3 * last)
        for n, cp in enumerate(cp_loop):
            if 3 + n * (n_iter - 4) // len(cp_loop) == g:
                cp.start()

    def project_ahead(g0, pairs, iters, i, carry):
        j0 = bounds[g0] + i * pairs
        for u in range(3 * pairs):
            k = 3 * j0 + u
            pltpu.make_async_copy(raw_v.at[k], raw_v.at[k], wsem.at[k]).wait()
        for c in range(iters):
            pl.when(i == c)(functools.partial(prefetch, g0 + c))
        for u in range(pairs):
            for m in range(3):
                j = j0 + u
                w = raw_v[3 * j + m]
                even = pltpu.bitcast(w << 16, F32).astype(BF16)
                odd = pltpu.bitcast(w & np.uint32(0xFFFF0000), F32).astype(BF16)
                for t, wt in enumerate((even, odd)):
                    hm = (2 * j + t) * 3 + m
                    w_v[hm] = pltpu.bitcast(wt, U32)
                    d = _mm(pltpu.bitcast(xan_v[...], BF16), wt)
                    pre_v[pl.ds(0, NSEG), pl.ds(pl.multiple_of(hm * AHEAD, AHEAD), AHEAD), :] = (
                        d.reshape(NSEG, AHEAD, Dh))
        return carry

    g0 = 0
    for pairs, iters in PHASES:
        lax.fori_loop(0, iters, functools.partial(project_ahead, g0, pairs, iters), 0)
        g0 += iters
    for cp in cp_loop:
        cp.wait()
    for cp in cp_ffn:
        cp.start()

    def ln_segment(s):
        v = yield from _layernorm(x_v[s].astype(F32))
        for n in range(NCOL):
            pre_v[s, pl.ds(XN + n * SEG, SEG), :] = v[:, n * LANES:(n + 1) * LANES]

    _finish(ln_segment(0))
    wr = wr_v[...].astype(F32).reshape(1, D)
    row_id = lax.broadcasted_iota(I32, (SEG, LANES), 0)

    def residual(s, live):
        r0 = pl.multiple_of(s * SEG, SEG)
        h = _rb(x_v[s].astype(F32) + _rb(att_v[...]))
        h_v[pl.ds(r0, SEG), :] = h
        hn = yield from _layernorm(h)
        hn_v[pl.ds(r0, SEG), :] = hn
        out_v[pl.ds(r0, SEG), :] = (h + hn).astype(BF16)
        r = jnp.broadcast_to(_rb(jnp.sum(hn * wr, axis=-1, keepdims=True)), (SEG, LANES))
        u = pltpu.bitcast(r, I32) >> 16
        rank = jnp.where(r == r, (u ^ ((u >> 15) & 0x7FFF)) + 0x8000, 0)
        key = jnp.where(live, rank * S + (S - 1 - r0) - row_id, -1)
        key = pltpu.bitcast(key + KEY_BASE, F32)
        yield
        best = top[0][...]
        top[0][...] = jnp.maximum(best, key)
        top[1][...] = jnp.maximum(top[1][...], jnp.minimum(best, key))

    groups = [range(a, min(a + G, H)) for a in range(0, H, G)]
    exp2_scale = scale * math.log2(math.e)

    def step(s, mem, deferred):
        xs = jnp.concatenate([pre_v[s, pl.ds(XN + n * SEG, SEG), :] for n in range(NCOL)], axis=1)
        lhs = jnp.concatenate([xs[AHEAD:], mem], axis=0).astype(BF16)
        qkv, probs, heads = {}, {}, {}
        acc_mem, acc_x = [None] * NCOL, [None] * NCOL
        next_ln = ln_segment(jnp.minimum(s + 1, NSEG - 1))
        prev = residual(jnp.maximum(s - 1, 0), s > 0)

        def project(g, m):
            for hd in groups[g]:
                d = _mm(lhs, pltpu.bitcast(w_v[hd * 3 + m], BF16))
                early = pre_v[s, pl.ds((hd * 3 + m) * AHEAD, AHEAD), :]
                qkv[hd, m] = jnp.concatenate([d[SEG - AHEAD:], early, d[:SEG - AHEAD]], axis=0)

        def stacked(g, m):
            return [qkv.pop((hd, m)) for hd in groups[g]]

        def tile(g, m):
            pad = jnp.zeros((LANES - len(groups[g]) * L, Dh), F32)
            return jnp.concatenate(stacked(g, m) + [pad], axis=0).astype(BF16)

        def scores(g):
            q = jnp.concatenate(stacked(g, 0), axis=0)
            sc = lax.dot_general(q, tile(g, 1), (((1,), (1,)), ((), ())), preferred_element_type=F32)
            cap = cap_v[pl.ds(0, q.shape[0]), :]
            sc = jnp.where(cap > 0.0, sc, cap)
            probs[g] = jnp.exp2((sc - jnp.max(sc, axis=-1, keepdims=True)) * exp2_scale)

        def attend(g):
            v = tile(g, 2)
            e = probs.pop(g)
            inv = pltpu.reciprocal(jnp.sum(e, axis=-1, keepdims=True), full_range=False)
            o = _mm(e, v) * inv
            for i, hd in enumerate(groups[g]):
                heads[hd] = o[i * L:(i + 1) * L]

        def output(hd, with_mem, with_x):
            o = heads[hd][(0 if with_mem else M):(L if with_x else M)]
            for n in range(NCOL):
                d = _mm(o, pltpu.bitcast(wo_v[n, pl.ds(hd * Dh // 2, Dh // 2), :], BF16))
                if with_mem:
                    acc_mem[n] = d[:M] if acc_mem[n] is None else acc_mem[n] + d[:M]
                if with_x:
                    acc_x[n] = d[-SEG:] if acc_x[n] is None else acc_x[n] + d[-SEG:]

        pending = list(range(H))

        def output_upto(end):
            while pending and pending[0] < end:
                hd = pending.pop(0)
                output(hd, True, hd not in deferred)

        ng = len(groups)
        for t in range(ng + 3):
            if t in RESIDUAL_SLOTS:
                next(prev, None)
            if t in NEXT_LN_SLOTS:
                next(next_ln, None)
            if t < ng:
                project(t, 0)
                project(t, 1)
            output_upto(WO_UPTO.get(t, (0, 0))[0])
            if 0 <= t - 1 < ng:
                scores(t - 1)
                project(t - 1, 2)
            output_upto(WO_UPTO.get(t, (0, 0))[1])
            if t >= 3:
                attend(t - 3)
        output_upto(H)
        for hd in deferred:
            output(hd, False, True)
        _finish(prev)
        _finish(next_ln)
        att_v[...] = jnp.concatenate(acc_x, axis=1)
        return jnp.concatenate(acc_mem, axis=1)

    flush_at = NSEG // UNROLL - 1
    done = (flush_at * UNROLL - 1) * SEG
    cp_head = new_copy(out_v.at[pl.ds(0, done)], out_hbm.at[pl.ds(0, done)])
    cp_tail = new_copy(out_v.at[pl.ds(done, S - done)], out_hbm.at[pl.ds(done, S - done)])

    def steps(i, mem):
        pl.when(i == flush_at)(cp_head.start)
        for u in range(UNROLL):
            mem = step(i * UNROLL + u, mem, DEFERRED_HEADS if u < UNROLL - 1 else ())
        return mem

    lax.fori_loop(0, NSEG // UNROLL, steps, mem0_v[...].astype(F32))

    for cp in cp_ffn:
        cp.wait()
    _finish(residual(NSEG - 1, True))
    cp_tail.start()

    best = top[0][...]
    k1 = jnp.max(best, axis=0, keepdims=True)
    k2 = jnp.max(jnp.where(best == k1, top[1][...], best), axis=0, keepdims=True)

    def token(key):
        key = pltpu.bitcast(jnp.broadcast_to(key, (8, LANES)), I32) - KEY_BASE
        return jnp.clip(S - 1 - lax.rem(key[0, 0], S), 0, S - 1)

    i1, i2 = token(k1), token(k2)
    first = lax.broadcasted_iota(I32, (8, D), 0) == 0
    h_sel = jnp.where(first, h_v[pl.ds(i1, 1), :], h_v[pl.ds(i2, 1), :])
    x_sel = jnp.where(first, hn_v[pl.ds(i1, 1), :], hn_v[pl.ds(i2, 1), :])
    gate = _rb(_mm(x_sel, wg_v[...]))
    up = _rb(_mm(x_sel, wu_v[...]))
    y = _rb(_mm(_rb(_rb(gate * _sigmoid(gate)) * up), wd_v[...]))
    r_sel = _rb(jnp.sum(x_sel * wr, axis=-1, keepdims=True))
    routed = h_sel + _rb(x_sel + _rb(y * _sigmoid(r_sel)))

    cp_head.wait()
    cp_tail.wait()
    row16 = lax.broadcasted_iota(I32, (16, D), 0)
    blocks = []
    for j, idx in enumerate((i1, i2)):
        b0 = pl.multiple_of((idx // 16) * 16, 16)
        cur = out_v[pl.ds(b0, 16), :].astype(F32)
        out_v[pl.ds(b0, 16), :] = jnp.where(row16 == idx - b0, routed[j:j + 1], cur).astype(BF16)
        blocks.append(b0)
    patch = [new_copy(out_v.at[pl.ds(b0, 16)], out_hbm.at[pl.ds(b0, 16)]) for b0 in blocks]
    patch[0].start()

    @pl.when(blocks[0] != blocks[1])
    def _():
        patch[1].start()
        patch[1].wait()

    patch[0].wait()


@functools.partial(jax.jit, static_argnames=("A_seg_len",))
def pallas_sequential_preLN__memory_aug_recurrent_mem_tr__moe_arch_mod__prompt_kernel(
    A_x: jax.Array,
    A_mem0: jax.Array,
    A_Wq: jax.Array,
    A_Wk: jax.Array,
    A_Wv: jax.Array,
    A_Wo: jax.Array,
    A_seg_len: int,
    B_x: jax.Array,
    B_w_r: jax.Array,
    B_w_gate: jax.Array,
    B_w_up: jax.Array,
    B_w_down: jax.Array,
):
    del B_x
    B, S, D = A_x.shape
    _, H, Dh = A_Wq.shape
    M = A_mem0.shape[1]
    F = B_w_gate.shape[1]
    SEG = A_seg_len
    NSEG = S // SEG
    L = M + SEG
    assert B == 1 and Dh == LANES and NSEG % UNROLL == 0

    hbm = pl.BlockSpec(memory_space=pl.ANY)
    out = pl.pallas_call(
        _kernel,
        out_shape=jax.ShapeDtypeStruct((S, D), BF16),
        in_specs=[hbm] * 10,
        out_specs=hbm,
        scratch_shapes=[
            pltpu.VMEM((M, D), BF16),
            pltpu.VMEM((D,), BF16),
            pltpu.VMEM((NSEG, AHEAD, D), BF16),
            pltpu.VMEM((NSEG * AHEAD // 2, D), U32),
            pltpu.VMEM((NSEG, SEG, D), BF16),
            pltpu.VMEM((3 * H // 2, D, Dh), U32),
            pltpu.VMEM((3 * H, D // 2, Dh), U32),
            pltpu.VMEM((NSEG + 1, 3 * H * AHEAD + SEG * D // LANES, Dh), F32),
            pltpu.VMEM((D // LANES, H * Dh // 2, LANES), U32),
            pltpu.VMEM((D, F), BF16),
            pltpu.VMEM((D, F), BF16),
            pltpu.VMEM((F, D), BF16),
            pltpu.VMEM((S, D), F32),
            pltpu.VMEM((S, D), F32),
            pltpu.VMEM((SEG, D), F32),
            pltpu.VMEM((LANES // L * L, LANES), F32),
            pltpu.VMEM((S, D), BF16),
            pltpu.SemaphoreType.DMA((3 * H // 2,)),
            pltpu.SemaphoreType.DMA((12 + D // LANES,)),
        ],
        compiler_params=pltpu.CompilerParams(vmem_limit_bytes=100 * 1024 * 1024),
        name="rmt_mod",
    )(A_x.reshape(NSEG, SEG, D), A_mem0.reshape(M, D), A_Wq, A_Wk, A_Wv, A_Wo.reshape(H * Dh, D),
      B_w_r, B_w_gate, B_w_up, B_w_down)
    return out.reshape(B, S, D)
```
